```python
import os as _os
_os.environ.setdefault("JAX_PLATFORMS", "cpu")
import jax
import jax.numpy as jnp

def _softmax(x, axis=-1):
    return jax.nn.softmax(x, axis=axis)
def _gelu(x):
    return jax.nn.gelu(x, approximate=True)
def _silu(x):
    return jax.nn.silu(x)
def _sigmoid(x):
    return jax.nn.sigmoid(x)
def _layernorm(x, axis=-1, eps=1e-5):
    m = jnp.mean(x, axis=axis, keepdims=True)
    v = jnp.var(x, axis=axis, keepdims=True)
    return (x - m) / jnp.sqrt(v + eps)
def _scatter_add(tgt, idx, src, axis=0):
    return tgt.at[idx].add(src)
def _segment_sum(src, seg, n):
    return jax.ops.segment_sum(src, seg, n)
class _Rng:
    def __init__(self, key):
        self._k = key
    def _next(self):
        self._k, sub = jax.random.split(self._k)
        return sub
    def normal(self, shape):
        return jax.random.normal(self._next(), shape, dtype=jnp.bfloat16)
    def randint(self, lo, hi, shape):
        return jax.random.randint(self._next(), shape, lo, hi, dtype=jnp.int32)
    def uniform(self, shape, lo=0.0, hi=1.0):
        return jax.random.uniform(self._next(), shape, jnp.bfloat16, lo, hi)
    def permutation(self, n):
        return jax.random.permutation(self._next(), n)


kernel_name = 'gated_mix__ssm_conv_h3__mixer_s_mlp__prompt'

def setup_inputs():
    _rng = _Rng(jax.random.key(int.from_bytes(__import__("os").urandom(4), "little")))
    _w = (lambda a: (lambda t: t.astype(jnp.bfloat16) if jnp.issubdtype(t.dtype, jnp.floating) else t)(jnp.asarray(a)))
    def _A_setup():
        B, S, D = 1, 2048, 576
        ks = 4
        return {
            "q": _w((lambda *s: _rng.normal(s) * 0.05)(B, S, D)),
            "k": _w((lambda *s: _rng.normal(s) * 0.4)(B, S, D)),
            "v": _w((lambda *s: _rng.normal(s) * 0.4)(B, S, D)),
            "shift_k": _w((lambda *s: _rng.normal(s) * 0.4)(D, ks) * 0.5),
            "ssm_k": _w((lambda *s: _rng.normal(s) * 0.4)(D, S) * (1.0 / S ** 0.5)),
            "ssm_D": _w((lambda *s: _rng.normal(s) * 0.4)(D)),
        }
    _A_in = _A_setup()

    def _B_setup():
        B, S, D, F = 1, 2048, 576, 4608
        return {
            "x":  _w((lambda *s: _rng.normal(s) * 0.05)(B, S, D)),
            "w1": _w((lambda *s: _rng.normal(s) * 0.2)(D, D) * (D ** -0.5)),
            "w2": _w((lambda *s: _rng.normal(s) * 0.2)(D, D) * (D ** -0.5)),
            "w3": _w((lambda *s: _rng.normal(s) * 0.2)(D, F) * (D ** -0.5)),
            "w4": _w((lambda *s: _rng.normal(s) * 0.2)(F, D) * (F ** -0.5)),
        }
    _B_in = _B_setup()

    return {
        "A_q": _A_in["q"],
        "A_k": _A_in["k"],
        "A_v": _A_in["v"],
        "A_shift_k": _A_in["shift_k"],
        "A_ssm_k": _A_in["ssm_k"],
        "A_ssm_D": _A_in["ssm_D"],
        "B_x": _B_in["x"],
        "B_w1": _B_in["w1"],
        "B_w2": _B_in["w2"],
        "B_w3": _B_in["w3"],
        "B_w4": _B_in["w4"],
        "gate_w": _w((lambda *s: _rng.normal(s) * 0.05)(576) * 16.0),
    }

def reference(A_q, A_k, A_v, A_shift_k, A_ssm_k, A_ssm_D, B_x, B_w1, B_w2, B_w3, B_w4, gate_w):
    def _A_ref(q, k, v, shift_k, ssm_k, ssm_D):
        B, S, D = q.shape
        ks = shift_k.shape[-1]
        k_pad = jnp.pad(k, ((0, 0), (ks - 1, 0), (0, 0)))
        k_shift = jnp.zeros_like(k)
        for t in range(ks):
            k_shift = k_shift + k_pad[:, t:t + S, :] * shift_k[:, ks - 1 - t][None, None, :]
        kv = k_shift * v
        L = 2 * S
        kv_pad = jnp.pad(kv, ((0, 0), (0, S), (0, 0)))
        kf_pad = jnp.pad(ssm_k, ((0, 0), (0, S)))
        kv_f = (lambda x, axes=(-2,-1): jnp.fft.rfft2(x.astype(jnp.float32), axes=axes))(kv_pad[:, None, :, :], axes=(1, 2))
        kf_f = (lambda x, axes=(-2,-1): jnp.fft.rfft2(x.astype(jnp.float32), axes=axes))(kf_pad[:, None, :], axes=(1, 2))
        kf_f = (lambda x, *d: x.transpose(*d))(kf_f, 1, 2, 0)
        y_f = kv_f * kf_f[None, :, :, :]
        y = (lambda x, s, axes=(-2,-1): jnp.fft.irfft2(x, s=s, axes=axes).astype(jnp.bfloat16))(y_f, (1, L), axes=(1, 2))[:, 0, :S, :]
        y = y + kv * ssm_D[None, None, :]
        return q * y

    def _B_ref(x, w1, w2, w3, w4):
        B, S, D = x.shape
        h = _gelu(_layernorm(x, axis=-1) @ w1)
        c = D // 4
        g0 = jnp.pad(h[:, :, 0*c:1*c], ((0, 0), (1, 0), (0, 0)))[:, :S, :]
        g1 = jnp.pad(h[:, :, 1*c:2*c], ((0, 0), (0, 1), (0, 0)))[:, 1:, :]
        g2 = jnp.pad(h[:, :, 2*c:3*c], ((0, 0), (2, 0), (0, 0)))[:, :S, :]
        g3 = jnp.pad(h[:, :, 3*c:   ], ((0, 0), (0, 2), (0, 0)))[:, 2:, :]
        hs = jnp.concatenate([g0, g1, g2, g3], axis=-1) @ w2
        x1 = x + hs
        h2 = _gelu(_layernorm(x1, axis=-1) @ w3) @ w4
        return x1 + h2

    x = A_q
    g = _sigmoid((x * gate_w).sum(-1, keepdims=True))
    a = _A_ref(x, A_k, A_v, A_shift_k, A_ssm_k, A_ssm_D)
    b = _B_ref(x, B_w1, B_w2, B_w3, B_w4)
    return g * a + (1 - g) * b
```

```python
import math

import jax
import jax.numpy as jnp
import numpy as np
import jax.experimental.pallas as pl
import jax.experimental.pallas.tpu as pltpu

D, S, F = 576, 2048, 4608
LANE = 128
ROW = 16
DC = D // ROW
UNIT = 4 * LANE
NUNIT = S // UNIT
QD = D // 4
FCH = 4 * LANE
NCH = F // FCH
FIRST = (0, 4, 8, 9)
PIECE = 32
NCONV = D // ROW
SHIFTS = (1, -1, 2, -2)
LN_EPS = 1e-5

f32, bf16, u32 = jnp.float32, jnp.bfloat16, jnp.uint32

_C0 = math.sqrt(2.0 / math.pi)
GELU_IN = (_C0 * 0.044715) ** (1.0 / 3.0)
GELU_A = _C0 / GELU_IN
GELU_OUT = 0.5 / GELU_IN

CFG = dict(
    back=180, early_back=200, lane_back=450, gap=45,
    rate=1.0, max_rate=2.5, margin=150, cool=150,
    room_up=(1, 1, 1, 0.8, 0.8, 0.6, 0.6), room_down=1.0, room_conv=0.5, room_square=1.1,
    late=24, conv=(64, 124), lag=2, outs=(2, 3, 4),
)
WORK = dict(up=2592, down=2520, x=3000, tokens=2160, conv_in=624, conv_mul=740)

_WEIGHTS = 55 * 8 + 49 * 9
_RING = 3
_SIZES = dict(weights=NCH * _WEIGHTS, tokens=NUNIT * 55 * 8, conv=_RING * 64, sums=8, spare=2)
_BASE = dict(zip(_SIZES, np.cumsum([0] + list(_SIZES.values())).tolist()))
_BASE["x"] = _BASE["weights"] + FIRST[1] * _WEIGHTS
_NCELL = sum(_SIZES.values())


def _dft_tables():
    lane = np.arange(LANE)
    fwd = []
    for rho in range(4):
        j = (lane - rho) % 4
        t = LANE * j + (lane - j) % LANE
        theta = 2.0 * np.pi * np.outer(t, 2.0 * lane + 0.5) / (2 * UNIT)
        fwd.append(np.concatenate([np.cos(theta), -np.sin(theta)], axis=1))
    fwd = np.stack(fwd)
    inv = fwd.transpose(0, 2, 1) / UNIT

    def words(a):
        half = np.ascontiguousarray(a.astype(np.float32).astype(bf16)).view(np.uint16).astype(np.uint32)
        return half[:, 0::2] | (half[:, 1::2] << 16)
    return words(fwd), words(inv)


_WF, _WI = _dft_tables()


def _gelu2(z):
    return z + z * jnp.tanh(z * (z * z + GELU_A))


def _lane_id(rows):
    return jax.lax.broadcasted_iota(jnp.int32, (rows, LANE), 1)


def _left(a11, a12, a21, a22):
    return [a11 + a22, a21 + a22, a11, a22, a11 + a12, a21 - a11, a12 - a22]


def _right(b11, b12, b21, b22):
    return [b11 + b22, b11, b12 - b22, b21 - b11, b22, b11 + b12, b21 + b22]


def _result(m):
    return [[m[0] + m[3] - m[4] + m[6], m[2] + m[4]],
            [m[1] + m[3], m[0] - m[1] + m[2] + m[5]]]


_LEFT = (((0, 0, 1), (1, 1, 1)), ((1, 0, 1), (1, 1, 1)), ((0, 0, 1),), ((1, 1, 1),), ((0, 0, 1), (0, 1, 1)),
         ((1, 0, 1), (0, 0, -1)), ((0, 1, 1), (1, 1, -1)))
_ORDER = (0, 6, 3, 4, 1, 2, 5)


def _collapse(group, extra=None):
    out = [[None] * 4 for _ in range(4)]

    def plus(z, r, c):
        add = extra(r, c) if extra else {}
        return [[z[i][j] + add[i, j] if (i, j) in add else z[i][j] for j in range(2)] for i in range(2)]

    def both(fn, a, b):
        return [[fn(a[i][j], b[i][j]) for j in range(2)] for i in range(2)]

    def emit(z, r, c):
        for i in range(2):
            for j in range(2):
                out[2 * i + r][2 * j + c] = z[i][j]

    y0 = group(0)
    first = both(jnp.add, plus(y0, 0, 0), group(6))
    y3 = group(3)
    first = both(jnp.add, first, y3)
    y4 = group(4)
    emit(both(jnp.subtract, first, y4), 0, 0)
    low = plus(y3, 1, 0)
    y1 = group(1)
    emit(both(jnp.add, low, y1), 1, 0)
    last = both(jnp.subtract, y0, y1)
    high = plus(y4, 0, 1)
    y2 = group(2)
    emit(both(jnp.add, high, y2), 0, 1)
    last = plus(both(jnp.add, last, y2), 1, 1)
    emit(both(jnp.add, last, group(5)), 1, 1)
    return out


def _left576(group, t):
    lo = _lane_id(ROW) < LANE // 2
    if group >= 7:
        r = group - 7
        u0, u2, v0, v2 = t(r, 0), t(r, 2), t(2 + r, 0), t(2 + r, 2)
        return [(49 + r, u0 + v2), (51 + r, jnp.where(lo, u2 - v2, t(r, 4))),
                (53 + r, jnp.where(lo, v0 - u0, t(2 + r, 4)))]
    pair = (lambda u, v: (v(0) + v(2), v(1) + v(3)),
            lambda u, v: (jnp.where(lo, u(0), v(2)), v(3)),
            lambda u, v: (jnp.where(lo, v(2), u(0)), u(1)),
            lambda u, v: (u(0) + u(2), u(1) + u(3)),
            lambda u, v: (jnp.where(lo, 0.0, u(0) + v(2)), u(1) + v(3)),
            lambda u, v: (jnp.where(lo, u(4), u(2) - v(2)), u(3) - v(3)),
            lambda u, v: (jnp.where(lo, v(4), v(0) - u(0)), v(1) - u(1)))[group]
    top, bottom = [pair(lambda k: t(r, k), lambda k: t(2 + r, k)) for r in range(2)]
    return [(7 * group + i, x) for i, x in enumerate(_left(*top, *bottom))]


def _right576(group, r, x):
    zero = jnp.zeros((ROW, LANE), f32)
    if group >= 7:
        c = group - 7
        if r >= 64:
            return [(49 + c, zero), (51 + c, x(c, 448 + r)), (53 + c, x(2 + c, 448 + r))]
        p1, q2 = x(c, r), x(2 + c, 256 + r)
        return [(49 + c, p1 + q2), (51 + c, x(c, 256 + r) + q2), (53 + c, p1 + x(2 + c, r))]

    def part(c, k):
        p1, p2, ps = [lambda d=d: x(c, d + k) for d in (0, 256, 512)]
        q1, q2, qs = [lambda d=d: x(2 + c, d + k) for d in (0, 256, 512)]
        if k < 64:
            return (p1, lambda: q1() - q2(), lambda: p2() - p1(), q2, lambda: None, qs, ps)[group]()
        return (lambda: -q1(), lambda: q2() - q1(), lambda: p1() - p2(), lambda: -p2(), lambda: q1() + p2(),
                lambda: p2() + q2(), lambda: p1() + q1())[group]()

    b11, b12, b21, b22 = part(0, r), part(1, r), part(0, LANE + r), part(1, LANE + r)
    out = [b22, zero, -b22, b21, b22, zero, b21 + b22] if b11 is None else _right(b11, b12, b21, b22)
    return [(7 * group + i, v) for i, v in enumerate(out)]


def _product576(mm):
    def group(b):
        x2, x3, x4, x5, xj, e12, e21 = [mm(7 * p + b, 7 * p + b, _ORDER.index(b)) for p in range(7)]
        return [[x4 - x5, (x3 + x5) + (xj + e12)], [(x2 + x4) + (xj + e21), x3 - x2]]

    def extra(r, c):
        xi, e11, e22 = [mm(49 + 2 * p + r, 49 + 2 * p + c, 0) for p in range(3)]
        return {(0, 0): xi + e11, (1, 1): xi + e22}

    return _collapse(group, extra)


def _left49(b, x):
    def inner(i, j):
        (r, c, _), *rest = _LEFT[b]
        v = x(2 * i + r, 2 * j + c)
        for r, c, sign in rest:
            v = v + x(2 * i + r, 2 * j + c) if sign > 0 else v - x(2 * i + r, 2 * j + c)
        return v
    return [(7 * a + b, v) for a, v in enumerate(_left(inner(0, 0), inner(0, 1), inner(1, 0), inner(1, 1)))]


def _right49(x):
    inner = [[_right(x[2 * i][2 * j], x[2 * i][2 * j + 1], x[2 * i + 1][2 * j], x[2 * i + 1][2 * j + 1])
              for j in range(2)] for i in range(2)]
    for b in (4, 6, 0, 1, 3, 2, 5):
        for a, v in enumerate(_right(inner[0][0][b], inner[0][1][b], inner[1][0][b], inner[1][1][b])):
            yield 7 * a + b, v


def _barrel(v):
    lane = _lane_id(v[0].shape[0])
    q = [v[(-p) % 4] for p in range(4)]
    q = [jnp.where((lane & 1) != 0, q[(p - 1) % 4], q[p]) for p in range(4)]
    return [jnp.where((lane & 2) != 0, q[(p - 2) % 4], q[p]) for p in range(4)]


def _split_phases(tiles):
    return _barrel([t if j == 0 else pltpu.roll(t, j, 1) for j, t in enumerate(tiles)])


def _merge_phases(phases):
    return [t if j == 0 else pltpu.roll(t, LANE - j, 1) for j, t in enumerate(_barrel(phases))]


def _dft4(u, sign):
    (r0, i0), (r1, i1), (r2, i2), (r3, i3) = u
    ar, ai, br, bi = r0 + r2, i0 + i2, r0 - r2, i0 - i2
    cr, ci, dr, di = r1 + r3, i1 + i3, r1 - r3, i1 - i3
    plus, minus = (br - di, bi + dr), (br + di, bi - dr)
    return [(ar + cr, ai + ci), plus if sign > 0 else minus, (ar - cr, ai - ci), minus if sign > 0 else plus]


def _make_kernel(cfg):
    def kernel(zero_ref, x_hbm, k_hbm, v_hbm, sk_hbm, ssm_hbm, sd_hbm, w1_hbm, w2_hbm, w3_hbm, w4_hbm, gw_hbm,
               wf_hbm, wi_hbm, out_hbm,
               k_v, v_v, sk_v, ssm_v, sd_v, w1_v, w2_v, w3_v, w4_v, gw_v, wf_v, wi_v, out_v, col_v, arena, sems,
               *buffers):
        x_v, shifted, normed, acc = [buffers[NUNIT * k:NUNIT * (k + 1)] for k in range(4)]
        square, hidden = buffers[4 * NUNIT:4 * NUNIT + 2], buffers[4 * NUNIT + 2:]

        copies = {}

        def copy(name, src, dst):
            copies[name] = pltpu.make_async_copy(src, dst, sems.at[len(copies)])

        def copy_x(u):
            copy(("x", u), x_hbm.at[:, pl.ds(u * UNIT, UNIT)], x_v[u])

        def copy_chunks(name, src, dst, first, last):
            cols = pl.ds(first * FCH, (last - first) * FCH)
            copy(name, src.at[:, cols], dst.at[:, cols])

        copy("sk", sk_hbm, sk_v)
        copy("sd", sd_hbm, sd_v)
        copy("gw", gw_hbm, gw_v)
        copy_x(0)
        copy("w1", w1_hbm, w1_v)
        for u in range(1, NUNIT):
            copy_x(u)
        copy("w2", w2_hbm, w2_v)
        copy_chunks("w3a", w3_hbm, w3_v, 0, FIRST[1])
        copy_chunks("w4a", w4_hbm, w4_v, 0, FIRST[1])
        copy_chunks("w3b", w3_hbm, w3_v, FIRST[1], NCH)
        copy_chunks("w4b", w4_hbm, w4_v, FIRST[1], NCH)
        copy("wf", wf_hbm, wf_v)
        copy("wi", wi_hbm, wi_v)
        copy("ssm", ssm_hbm, ssm_v.at[pl.ds(0, D)])
        copy("k", k_hbm, k_v.at[pl.ds(0, D)])
        copy("v", v_hbm, v_v)
        for c in copies.values():
            c.start()
        for first, last in zip((0,) + cfg["outs"], cfg["outs"]):
            cols = pl.ds(first * UNIT, (last - first) * UNIT)
            copy(("out", last), out_v.at[:, cols], out_hbm.at[:, cols])

        def wait(*names):
            for name in names:
                copies[name].wait()

        words = arena.bitcast(u32)
        zero = jnp.clip(zero_ref[0], 0, 1)
        val, jobs, recent = {}, [], []
        clock = dict(now=0.0, room=0.0, budget=0.0, cool=0.0, pinned=0.0, pending=False, slot=0)

        def tile(j):
            return slice(j * LANE, (j + 1) * LANE)

        def put(cell, x):
            arena[cell] = x.astype(bf16)

        def as_bf16(w):
            return pltpu.bitcast(w.reshape(w.shape[0] * ROW // 2, LANE), bf16)

        def seal(ref, back=None):
            early = cfg["early_back"] if clock["now"] < 23500 else 0
            due = clock["now"] - (back or cfg["back"]) - early
            mark = jnp.zeros((8, LANE), f32)
            for t, m, r in reversed(recent):
                if t <= due:
                    mark = m[r:r + 8, :LANE]
                    break
            view = ref if ref.dtype == f32 else ref.bitcast(f32)
            if len(ref.shape) == 2:
                view[pl.ds(pl.multiple_of(view.shape[0] - ROW + 8 * zero, 8), 8), 0:LANE] = mark
            elif ref.shape[1] > ROW:
                view[ref.shape[0] - 1, pl.ds(pl.multiple_of(8 * zero, 8), 8), :] = mark
            else:
                view[ref.shape[0] - 2 + zero] = mark

        def step(job):
            cost = next(job["steps"], None)
            if cost is None:
                jobs.remove(job)
            else:
                clock["budget"] -= cost
                job["left"] -= cost
                clock["pending"] = True

        def finish_jobs(names):
            for job in [j for j in jobs if j["name"] in names]:
                while job in jobs:
                    step(job)
            clock["budget"] = max(clock["budget"], 0.0)

        def tick(cycles, weight, calm=True):
            hot = min(cycles, max(clock["cool"], 0.0))
            clock["cool"] -= cycles
            clock["now"] += cycles
            room = weight * (cycles - hot)
            rate, work = cfg["rate"], 0
            for job in sorted(jobs, key=lambda j: j["due"]):
                work += job["left"]
                rate = max(rate, work / max(room_before[job["due"][0]] - clock["room"] - cfg["margin"], 1.0))
            clock["room"] += room
            clock["budget"] = min(clock["budget"] + min(rate, cfg["max_rate"]) * room, 30.0)
            while clock["budget"] > 0:
                ready = [j for j in jobs if (calm and clock["cool"] < 0) or j["name"][0] != "conv_mul"]
                if not ready:
                    break
                step(min(ready, key=lambda j: j["due"]))

        def mm(lhs, rhs, weight, width=1, calm=True, turn=False):
            n, start = lhs[0][1], clock["now"]
            cycles = ROW * len(lhs) * width / 4
            pinned = {}
            for j in range(n):
                tick(cycles, weight, calm)
                if clock["pending"] and clock["now"] >= clock["pinned"] + cfg["gap"]:
                    k = j % len(lhs)
                    pinned[k, j] = words[pl.ds(lhs[k][0] + j + zero, 1)]
                    clock["pinned"], clock["pending"] = clock["now"], False
            tiles = []
            for k, (cell, _) in enumerate(lhs):
                parts, j0 = [], 0
                for j in sorted(j for t, j in pinned if t == k):
                    parts += [words[cell + j0:cell + j]] if j > j0 else []
                    parts.append(pinned[k, j])
                    j0 = j + 1
                parts += [words[cell + j0:cell + n]] if n > j0 else []
                tiles.append(as_bf16(parts[0] if len(parts) == 1 else jnp.concatenate(parts, axis=0)))
            a = tiles[0] if len(tiles) == 1 else jnp.concatenate(tiles, axis=1)
            m = jax.lax.dot_general(a, rhs(), (((1,), (int(turn),)), ((), ())), preferred_element_type=f32)
            recent.extend((start + j * cycles, m, j * ROW) for j in range(n))
            return m

        def up_cell(c, i):
            return _BASE["weights"] + _WEIGHTS * c + 8 * i

        def down_cell(c, i):
            return up_cell(c, 55) + 9 * i

        def prep_square(src, which):
            tail = src[4 * LANE:D, :]
            tiles = [src[k * LANE:(k + 1) * LANE, :] for k in range(4)] + [jnp.concatenate([tail, tail], axis=0)]
            for k, t in enumerate(tiles):
                square[which][D // 2 * k:D // 2 * (k + 1)] = pltpu.bitcast(t.T, u32)

        def prep_up(c):
            for r in range(0, LANE, ROW):
                for group in range(9):
                    for i, x in _right576(group, r, lambda j, k: w3_v[k:k + ROW, tile(4 * c + j)].astype(f32)):
                        put(up_cell(c, i) + r // ROW, x)
                    yield 36

        def prep_down(c):
            for r in range(0, QD, ROW):
                for b in _ORDER:
                    for i, x in _left49(b, lambda i, j: w4_v[
                            i * QD + r:i * QD + r + ROW, tile(4 * c + (j ^ 1))].astype(f32)):
                        put(down_cell(c, i) + r // ROW, x)
                    yield 40

        def columns(which):
            rows = [sk_v[...].astype(f32)[j:j + 1] for j in range(4)]
            rows += [sd_v[...].astype(f32).reshape(1, D), gw_v[...].astype(f32).reshape(1, D)]
            for j in which:
                col_v[j] = jnp.broadcast_to(rows[j], (LANE, D)).T

        def x_rows(u, j, r, n=ROW):
            return x_v[u][r:r + n, tile(j)].astype(f32)

        def prep_x(u):
            stats = []
            for slot, cost in enumerate((270, 230)):
                total = None
                for r in range(0, D, ROW):
                    term = [jnp.square(x_rows(u, j, r) - stats[0][j]) if stats else x_rows(u, j, r) for j in range(4)]
                    if not stats:
                        if r % QD == 0:
                            seal(col_v)
                        term += [t * col_v[5, r:r + ROW] for t in term]
                    total = term if total is None else [a + t for a, t in zip(total, term)]
                    if (r + ROW) % QD == 0:
                        for k in range(0, len(total), 4):
                            put(_BASE["sums"] + slot + k, (total[k] + total[k + 1]) + (total[k + 2] + total[k + 3]))
                        yield cost
                sums = [jnp.sum(a, axis=0, keepdims=True) for a in total]
                stats.append([a * (1.0 / D) for a in sums[:4]])
                for j, logit in enumerate(sums[4:]):
                    g = jax.nn.sigmoid(logit)
                    val["gate", 4 * u + j] = g
                    val["rest", 4 * u + j] = 1.0 - g
                    val["out", 4 * u + j] = (1.0 - g) * GELU_OUT
            scale = [jax.lax.rsqrt(v + LN_EPS) * GELU_IN for v in stats[1]]
            shift = [m * s for m, s in zip(stats[0], scale)]
            for r in range(0, D, ROW):
                for j in range(4):
                    put(_BASE["x"] + DC * (4 * (u % 2) + j) + r // ROW, x_rows(u, j, r) * scale[j] - shift[j])
                yield 28

        def square_product(which, source, cell):
            lhs, out = square[which], [[None] * 4 for _ in range(4)]
            for j in range(4):
                for i in range(4):
                    a = pltpu.bitcast(jnp.concatenate(
                        [lhs[(D * k + QD * i) // 2:(D * k + QD * (i + 1)) // 2] for k in range(5)], axis=1), bf16)
                    start, parts = clock["now"], []
                    for k in range(0, DC, 6):
                        tick(5 * QD / 4 / 6, cfg["room_square"])
                        first = cell + DC * j + k
                        if clock["pending"] and source is words:
                            parts += [words[pl.ds(first + zero, 1)], words[first + 1:first + 6]]
                            clock["pending"] = False
                        else:
                            parts.append(source[first:first + 6])
                    m = jnp.dot(a[:, :D], as_bf16(jnp.concatenate(parts, axis=0)), preferred_element_type=f32)
                    recent.extend((start + r * 5 / 4, m, r) for r in range(0, QD, ROW))
                    out[i][j] = m
            return out

        def mix_in(u):
            seal(arena)
            h = square_product(0, words, _BASE["x"] + 4 * DC * (u % 2))
            lane = _lane_id(QD)

            def keep(u, j, i, x):
                shifted[u][DC * j + 9 * i:DC * j + 9 * (i + 1)] = x.astype(bf16).reshape(9, ROW, LANE)

            for i, n in enumerate(SHIFTS):
                rolled = [pltpu.roll(_gelu2(z), n % LANE, 1) for z in h[i]]
                if n > 0:
                    for j in range(4):
                        before = rolled[j - 1] if j else val.get(("edge", i), 0.0)
                        keep(u, j, i, jnp.where(lane >= n, rolled[j], before))
                else:
                    if u > 0:
                        keep(u - 1, 3, i, jnp.where(lane < LANE + n, val["edge", i], rolled[0]))
                    for j in range(3 if u < NUNIT - 1 else 4):
                        keep(u, j, i, jnp.where(lane < LANE + n, rolled[j], rolled[j + 1] if j < 3 else 0.0))
                val["edge", i] = rolled[3]

        def mix_out(u):
            seal(arena)
            seal(shifted[u])
            y = square_product(1, shifted[u].bitcast(u32), 0)
            for j in range(4):
                x1, first, second = [], None, None
                for r in range(0, D, ROW):
                    i, k = divmod(r, QD)
                    x1.append(x_rows(u, j, r) + GELU_OUT * y[i][j][k:k + ROW])
                    pilot = x1[0][:1] if r == 0 else pilot
                    d = x1[-1] - pilot
                    first = d if first is None else first + d
                    second = d * d if second is None else second + d * d
                offset = jnp.sum(first, axis=0, keepdims=True) * (1.0 / D)
                var = jnp.maximum(jnp.sum(second, axis=0, keepdims=True) * (1.0 / D) - offset * offset, 0.0)
                scale = jax.lax.rsqrt(var + LN_EPS) * GELU_IN
                shift = (pilot + offset) * scale
                normal = [z * scale - shift for z in x1]
                for r, z in enumerate(x1):
                    val["skip", 4 * u + j, r] = val["rest", 4 * u + j] * z
                for k in range(5):
                    rows = normal[8 * k:8 * k + 8] if k < 4 else normal[32:] * 2
                    normed[u][5 * j + k] = jnp.concatenate(rows, axis=0).T

        def token_cell(u, i):
            return _BASE["tokens"] + 8 * (55 * u + i)

        def prep_tokens(u):
            for r in range(0, LANE, ROW):
                for group in range(9):
                    if group % 3 == 0:
                        seal(normed[u])
                    for i, x in _left576(group, lambda i, k: normed[u][5 * i + k, r:r + ROW]):
                        put(token_cell(u, i) + r // ROW, x)
                    yield 30

        def up(n, s, u, c, r):
            h = _product576(lambda a, b, k: mm([(token_cell(u, a) + r // ROW, PIECE // ROW)],
                                               lambda: as_bf16(words[up_cell(c, b):up_cell(c, b) + 8]),
                                               cfg["room_up"][k], calm=False))
            g = [[_gelu2(h[j][i ^ 1]) for j in range(4)] for i in range(4)]
            for k in range(0, PIECE, ROW):
                for p, x in _right49([[z[k:k + ROW] for z in row] for row in g]):
                    hidden[n % 2][8 * (49 * (c - FIRST[s]) + p) + (r + k) // ROW] = x.astype(bf16)
            clock["cool"] = cfg["cool"] * PIECE / 64

        def down(n, s, u, p):
            chunks = range(FIRST[s], FIRST[s + 1])
            source = hidden[n % 2].bitcast(u32)
            if p == 0:
                seal(source)
                if s > 0:
                    seal(acc[u])
            m = mm([(down_cell(c, p), 9) for c in chunks],
                   lambda: jnp.concatenate([as_bf16(source[8 * (49 * k + p):8 * (49 * k + p + 1)])
                                            for k in range(len(chunks))], axis=1), cfg["room_down"], turn=True)
            if s > 0:
                m = m + acc[u][p]
            if FIRST[s + 1] == NCH:
                val["acc", u, p] = m
            else:
                acc[u][p] = m

        def finish(u):
            for r in range(0, QD, ROW):
                y = _collapse(lambda b: _result([val["acc", u, 7 * a + b][r:r + ROW] for a in range(7)]))
                for i in range(4):
                    for j in range(4):
                        t, row = 4 * u + j, i * QD + r
                        base = jnp.concatenate([val["base", t, row], val["base", t, row + 8]], axis=0)
                        out_v[row:row + ROW, tile(t)] = (base + val["out", t] * y[i][j]).astype(bf16)
            if u + 1 in cfg["outs"]:
                copies["out", u + 1].start()

        def conv_cell(n, kind, rho):
            return _BASE["conv"] + 64 * (n % _RING) + 16 * kind + 4 * rho

        def conv_inputs(n):
            rows = slice(n * ROW, (n + 1) * ROW)
            lane = _lane_id(ROW // 2)
            seal(col_v, cfg["lane_back"])
            col = [col_v[j, rows] for j in range(4)]
            prev = [jnp.zeros((ROW // 2, LANE), u32)] * 3
            for i in range(NUNIT):
                seal(ssm_v, cfg["lane_back"])
                taps = _split_phases([pltpu.bitcast(ssm_v[rows, tile(4 * i + j)], u32) for j in range(4)])
                for rho in range(4):
                    words[conv_cell(n, 0, rho) + i] = taps[rho]
                yield 16
                seal(k_v, cfg["lane_back"])
                kv = []
                for t in range(4 * i, 4 * i + 4):
                    key = k_v[rows, tile(t)]
                    rolled = [pltpu.roll(pltpu.bitcast(key, u32), j, 1) for j in (1, 2, 3)]
                    total = key.astype(f32) * col[0]
                    for j in (1, 2, 3):
                        late = jnp.where(lane >= j, rolled[j - 1], prev[j - 1])
                        total = total + pltpu.bitcast(late, bf16).astype(f32) * col[j]
                    prev = rolled
                    kv.append(total * v_v[rows, tile(t)].astype(f32))
                    if t % 4 == 1:
                        yield 60
                for rho, x in enumerate(_split_phases(kv)):
                    put(conv_cell(n, 1, rho) + i, x)
                yield 80

        def conv_forward(n, kind):
            seal(arena)
            last = None
            for i in range(0, NUNIT, 2):
                u = {rho: mm([(conv_cell(n, kind, rho) + i, 2)], lambda: pltpu.bitcast(wf_v[rho], bf16),
                             cfg["room_conv"], 2) for rho in (0, 2, 1, 3)}
                for k in range(2):
                    rows = slice(k * ROW, (k + 1) * ROW)
                    z = [(u[rho][rows, :LANE], u[rho][rows, LANE:]) for rho in range(4)]
                    if kind == 0:
                        if last is None:
                            z[0] = (z[0][0] + col_v[4, n * ROW:(n + 1) * ROW], z[0][1])
                        z, last = z if last is None else [(a[0] - b[1], a[1] + b[0]) for a, b in zip(z, last)], z
                    val["spectrum", n, kind, i + k] = _dft4(z, -1)

        pairs = ((0, 3), (1, 2))

        def conv_multiply(n):
            for r in range(0, ROW, 8):
                def product(i, s):
                    re = im = None
                    for j in range(i + 1):
                        xr, xi = [z[r:r + 8] for z in val["spectrum", n, 1, j][s]]
                        kr, ki = [z[r:r + 8] for z in val["spectrum", n, 0, i - j][s]]
                        re = (xr * kr if re is None else re + xr * kr) - xi * ki
                        im = (xr * ki if im is None else im + xr * ki) + xi * kr
                    return re, im

                for h, pair in enumerate(pairs):
                    a, b = [_dft4([product(i, s) for s in range(4)], 1) for i in pair]
                    for rho in range(4):
                        for part in range(2):
                            put(conv_cell(n, 2 + part, rho) + r // 4 + h,
                                jnp.concatenate([a[rho][part], b[rho][part]], axis=0))
                    yield 185

        def conv_inverse(n):
            seal(arena)
            for k in range(2):
                ys = [mm([(conv_cell(n, 2 + part, rho) + 2 * k, 2) for part in range(2)],
                         lambda: pltpu.bitcast(wi_v[rho], bf16), cfg["room_conv"]) for rho in range(4)]
                row = n * ROW + 8 * k
                for q, i in enumerate(pairs[0] + pairs[1]):
                    y = _merge_phases([m[8 * q:8 * q + 8] for m in ys])
                    for j in range(4):
                        t = 4 * i + j
                        val["base", t, row] = ((val["gate", t] * y[j]) * x_rows(i, j, row, 8)
                                               + val["skip", t, n][8 * k:8 * k + 8])

        def job(kind, i):
            make = dict(x=prep_x, tokens=prep_tokens, up=prep_up, down=prep_down,
                        conv_in=conv_inputs, conv_mul=conv_multiply)[kind]
            return (kind, i), lambda: make(i)

        room = cfg["room_square"] * 20 * QD

        def first_stage(u, *frees):
            return lambda: mix_in(u), [("x", u)], frees, room

        def second_stage(u):
            return lambda: mix_out(u), (), [job("tokens", u)], room

        stream = [
            (lambda: wait("sk", "sd", "gw"), (), (), 0),
            (lambda: columns((5,)), (), (), 0),
            (lambda: wait(("x", 0)), (), [job("x", 0)], 0),
            (lambda: wait("w1"), [("x", 0)], (), 0),
            (lambda: prep_square(w1_v, 0), (), (), 0),
            (lambda: wait(("x", 1)), (), [job("x", 1)], 0),
            first_stage(0),
            (lambda: wait(("x", 2), ("x", 3)), (), [job("x", 2)], 0),
            first_stage(1, job("x", 3)),
            first_stage(2),
            (lambda: (wait("w2", "w3a"), prep_square(w2_v, 1)), (), [job("up", c) for c in range(FIRST[1])], 0),
            first_stage(3),
            second_stage(0),
            (lambda: wait("w4a"), (), [job("down", c) for c in range(FIRST[1])], 0),
            second_stage(1),
            second_stage(2),
            second_stage(3),
        ]

        slots = [(s, u) for s in range(len(FIRST) - 1) for u in range(NUNIT)]
        plan, begin = [], []
        for n, (s, u) in enumerate(slots):
            begin.append(len(plan))
            for c in range(FIRST[s], FIRST[s + 1]):
                for r in range(0, LANE, PIECE):
                    plan.append((len(plan) + 0.25, (
                        lambda n=n, s=s, u=u, c=c, r=r: up(n, s, u, c, r), [("up", c), ("tokens", u)], (),
                        (12 * cfg["room_up"][0] + 7 * sum(cfg["room_up"])) * PIECE / 4 - cfg["cool"] * PIECE / 64)))
        begin += [len(plan), len(plan) + 1]
        for n, (s, u) in enumerate(slots):
            count = begin[n + 2] - begin[n + 1]
            for k, p in enumerate(7 * a + b for b in _ORDER for a in range(7)):
                plan.append((begin[n + 1] + (k * count) // 49 + 0.75, (
                    lambda n=n, s=s, u=u, p=p: down(n, s, u, p),
                    [("down", c) for c in range(FIRST[s], FIRST[s + 1])] if k == 0 else (), (),
                    cfg["room_down"] * (FIRST[s + 1] - FIRST[s]) * QD / 4)))
            if FIRST[s + 1] == NCH:
                plan.append((begin[n + 2] - 0.2, (lambda u=u: finish(u), (), (), 0)))
        plan.append((cfg["late"] + 0.1, (
            lambda: (wait("w3b", "w4b", "wf", "wi", "ssm", "k", "v"), columns(range(5))), (),
            [job(kind, c) for c in range(FIRST[1], NCH) for kind in ("up", "down")]
            + [job("conv_in", n) for n in range(2)], 0)))
        for n in range(NCONV):
            pos = round(cfg["conv"][0] + (cfg["conv"][1] - cfg["conv"][0]) * n / NCONV)
            room = cfg["room_conv"] * 8 * ROW
            frees = [job("conv_mul", n)] + [job("conv_in", m) for m in (n + 2,) if m < NCONV]
            plan += [(pos + 0.9, (lambda n=n: conv_forward(n, 0), [("conv_in", n)], (), room)),
                     (pos + 0.91, (lambda n=n: conv_forward(n, 1), (), frees, room)),
                     (pos + cfg["lag"] + 0.89, (lambda n=n: conv_inverse(n), [("conv_mul", n)], (), room))]
        plan.sort(key=lambda e: e[0])
        stream += [e[1] for e in plan]

        due, room_before = {}, [0.0]
        for k, (_, needs, _, room) in enumerate(stream):
            room_before.append(room_before[-1] + room)
            for name in needs:
                due.setdefault(name, k)
        for name in due:
            if name[0] in ("up", "down"):
                due[name] = min(due[name], due["conv_in", 0])
        for k, (task, needs, frees, _) in enumerate(stream):
            clock["room"] = room_before[k]
            finish_jobs(needs)
            task()
            for name, make in frees:
                jobs.append(dict(name=name, steps=make(), due=(due[name], len(jobs)), left=WORK[name[0]]))
        wait(*[("out", last) for last in cfg["outs"]])

    return kernel


def make_fn(cfg):
    def fn(A_q, A_k, A_v, A_shift_k, A_ssm_k, A_ssm_D, B_x, B_w1, B_w2, B_w3, B_w4, gate_w):
        del B_x

        def feature_major(a):
            return jnp.swapaxes(a, 1, 2).reshape(D, S)

        args = (feature_major(A_q), feature_major(A_k), feature_major(A_v), A_shift_k.T, A_ssm_k, A_ssm_D,
                B_w1, B_w2, B_w3, B_w4.T, gate_w, jnp.asarray(_WF), jnp.asarray(_WI))
        plain = pltpu.VMEM((D, S), bf16)
        marked = pltpu.VMEM((D + 2 * ROW, S), bf16)
        out = pl.pallas_call(
            _make_kernel(cfg),
            out_shape=jax.ShapeDtypeStruct((D, S), bf16),
            in_specs=[pl.BlockSpec(memory_space=pltpu.SMEM)] + [pl.BlockSpec(memory_space=pl.ANY)] * len(args),
            out_specs=pl.BlockSpec(memory_space=pl.ANY),
            scratch_shapes=[
                marked, plain, pltpu.VMEM((4, D), bf16), marked, pltpu.VMEM((D,), bf16),
                pltpu.VMEM((D, D), bf16), pltpu.VMEM((D, D), bf16),
                pltpu.VMEM((D, F), bf16), pltpu.VMEM((D, F), bf16), pltpu.VMEM((D,), bf16),
                pltpu.VMEM(_WF.shape, u32), pltpu.VMEM(_WI.shape, u32), plain,
                pltpu.VMEM((6 + 1, D, LANE), f32),
                pltpu.VMEM((_NCELL, ROW, LANE), bf16),
                pltpu.SemaphoreType.DMA((14 + NUNIT + len(cfg["outs"]),)),
                *[pltpu.VMEM((D, UNIT), bf16)] * NUNIT,
                *[pltpu.VMEM((4 * DC + 2, ROW, LANE), bf16)] * NUNIT,
                *[pltpu.VMEM((20 + 1, LANE, LANE), f32)] * NUNIT,
                *[pltpu.VMEM((49 + 1, QD, LANE), f32)] * NUNIT,
                *[pltpu.VMEM((5 * D // 2, LANE), u32)] * 2,
                *[pltpu.VMEM((4 * 49 * 8 + 2, ROW, LANE), bf16)] * 2,
            ],
            compiler_params=pltpu.CompilerParams(vmem_limit_bytes=127 * 1024 * 1024),
            name="mlp_gated_mix",
        )(jnp.asarray(np.zeros((1,), np.int32)), *args)
        return jnp.swapaxes(out.reshape(1, D, S), 1, 2)
    return fn


@jax.jit
def pallas_gated_mix__ssm_conv_h3__mixer_s_mlp__prompt_kernel(
    A_q, A_k, A_v, A_shift_k, A_ssm_k, A_ssm_D, B_x, B_w1, B_w2, B_w3, B_w4, gate_w,
):
    return make_fn(CFG)(A_q, A_k, A_v, A_shift_k, A_ssm_k, A_ssm_D, B_x, B_w1, B_w2, B_w3, B_w4, gate_w)
```

```python
import math

import jax
import jax.numpy as jnp
import numpy as np
import jax.experimental.pallas as pl
import jax.experimental.pallas.tpu as pltpu

D, S, F = 576, 2048, 4608
LANE = 128
ROW = 16
DC = D // ROW
UNIT = 4 * LANE
NUNIT = S // UNIT
QD = D // 4
FCH = 4 * LANE
NCH = F // FCH
FIRST = (0, 4, 8, 9)
PIECE = 32
NCONV = D // ROW
SHIFTS = (1, -1, 2, -2)
LN_EPS = 1e-5

f32, bf16, u32 = jnp.float32, jnp.bfloat16, jnp.uint32

_C0 = math.sqrt(2.0 / math.pi)
GELU_IN = (_C0 * 0.044715) ** (1.0 / 3.0)
GELU_A = _C0 / GELU_IN
GELU_OUT = 0.5 / GELU_IN

CFG = dict(
    back=180, early_back=200, lane_back=450, gap=40,
    rate=1.0, max_rate=2.5, margin=150, cool=150,
    room_up=(1, 1, 1, 0.8, 0.8, 0.6, 0.6), room_down=1.0, room_conv=0.5, room_square=1.1,
    down_ready=13, late=24, conv=(64, 124), lag=2, outs=(2, 3, 4),
)
WORK = dict(up=2592, down=2520, x=3000, tokens=2160, conv_in=624, conv_mul=740)

_WEIGHTS = 55 * 8 + 49 * 9
_RING = 3
_SIZES = dict(weights=NCH * _WEIGHTS, tokens=NUNIT * 55 * 8, conv=_RING * 64, sums=8, spare=2)
_BASE = dict(zip(_SIZES, np.cumsum([0] + list(_SIZES.values())).tolist()))
_BASE["x"] = _BASE["weights"] + FIRST[1] * _WEIGHTS
_NCELL = sum(_SIZES.values())


def _dft_tables():
    lane = np.arange(LANE)
    fwd = []
    for rho in range(4):
        j = (lane - rho) % 4
        t = LANE * j + (lane - j) % LANE
        theta = 2.0 * np.pi * np.outer(t, 2.0 * lane + 0.5) / (2 * UNIT)
        fwd.append(np.concatenate([np.cos(theta), -np.sin(theta)], axis=1))
    fwd = np.stack(fwd)
    inv = fwd.transpose(0, 2, 1) / UNIT

    def words(a):
        half = np.ascontiguousarray(a.astype(np.float32).astype(bf16)).view(np.uint16).astype(np.uint32)
        return half[:, 0::2] | (half[:, 1::2] << 16)
    return words(fwd), words(inv)


_WF, _WI = _dft_tables()


def _gelu2(z):
    return z + z * jnp.tanh(z * (z * z + GELU_A))


def _lane_id(rows):
    return jax.lax.broadcasted_iota(jnp.int32, (rows, LANE), 1)


def _left(a11, a12, a21, a22):
    return [a11 + a22, a21 + a22, a11, a22, a11 + a12, a21 - a11, a12 - a22]


def _right(b11, b12, b21, b22):
    return [b11 + b22, b11, b12 - b22, b21 - b11, b22, b11 + b12, b21 + b22]


def _result(m):
    return [[m[0] + m[3] - m[4] + m[6], m[2] + m[4]],
            [m[1] + m[3], m[0] - m[1] + m[2] + m[5]]]


_LEFT = (((0, 0, 1), (1, 1, 1)), ((1, 0, 1), (1, 1, 1)), ((0, 0, 1),), ((1, 1, 1),), ((0, 0, 1), (0, 1, 1)),
         ((1, 0, 1), (0, 0, -1)), ((0, 1, 1), (1, 1, -1)))
_ORDER = (0, 6, 3, 4, 1, 2, 5)


def _collapse(group, extra=None):
    out = [[None] * 4 for _ in range(4)]

    def plus(z, r, c):
        add = extra(r, c) if extra else {}
        return [[z[i][j] + add[i, j] if (i, j) in add else z[i][j] for j in range(2)] for i in range(2)]

    def both(fn, a, b):
        return [[fn(a[i][j], b[i][j]) for j in range(2)] for i in range(2)]

    def emit(z, r, c):
        for i in range(2):
            for j in range(2):
                out[2 * i + r][2 * j + c] = z[i][j]

    y0 = group(0)
    first = both(jnp.add, plus(y0, 0, 0), group(6))
    y3 = group(3)
    first = both(jnp.add, first, y3)
    y4 = group(4)
    emit(both(jnp.subtract, first, y4), 0, 0)
    low = plus(y3, 1, 0)
    y1 = group(1)
    emit(both(jnp.add, low, y1), 1, 0)
    last = both(jnp.subtract, y0, y1)
    high = plus(y4, 0, 1)
    y2 = group(2)
    emit(both(jnp.add, high, y2), 0, 1)
    last = plus(both(jnp.add, last, y2), 1, 1)
    emit(both(jnp.add, last, group(5)), 1, 1)
    return out


def _left576(group, t):
    lo = _lane_id(ROW) < LANE // 2
    if group >= 7:
        r = group - 7
        u0, u2, v0, v2 = t(r, 0), t(r, 2), t(2 + r, 0), t(2 + r, 2)
        return [(49 + r, u0 + v2), (51 + r, jnp.where(lo, u2 - v2, t(r, 4))),
                (53 + r, jnp.where(lo, v0 - u0, t(2 + r, 4)))]
    pair = (lambda u, v: (v(0) + v(2), v(1) + v(3)),
            lambda u, v: (jnp.where(lo, u(0), v(2)), v(3)),
            lambda u, v: (jnp.where(lo, v(2), u(0)), u(1)),
            lambda u, v: (u(0) + u(2), u(1) + u(3)),
            lambda u, v: (jnp.where(lo, 0.0, u(0) + v(2)), u(1) + v(3)),
            lambda u, v: (jnp.where(lo, u(4), u(2) - v(2)), u(3) - v(3)),
            lambda u, v: (jnp.where(lo, v(4), v(0) - u(0)), v(1) - u(1)))[group]
    top, bottom = [pair(lambda k: t(r, k), lambda k: t(2 + r, k)) for r in range(2)]
    return [(7 * group + i, x) for i, x in enumerate(_left(*top, *bottom))]


def _right576(group, r, x):
    zero = jnp.zeros((ROW, LANE), f32)
    if group >= 7:
        c = group - 7
        if r >= 64:
            return [(49 + c, zero), (51 + c, x(c, 448 + r)), (53 + c, x(2 + c, 448 + r))]
        p1, q2 = x(c, r), x(2 + c, 256 + r)
        return [(49 + c, p1 + q2), (51 + c, x(c, 256 + r) + q2), (53 + c, p1 + x(2 + c, r))]

    def part(c, k):
        p1, p2, ps = [lambda d=d: x(c, d + k) for d in (0, 256, 512)]
        q1, q2, qs = [lambda d=d: x(2 + c, d + k) for d in (0, 256, 512)]
        if k < 64:
            return (p1, lambda: q1() - q2(), lambda: p2() - p1(), q2, lambda: None, qs, ps)[group]()
        return (lambda: -q1(), lambda: q2() - q1(), lambda: p1() - p2(), lambda: -p2(), lambda: q1() + p2(),
                lambda: p2() + q2(), lambda: p1() + q1())[group]()

    b11, b12, b21, b22 = part(0, r), part(1, r), part(0, LANE + r), part(1, LANE + r)
    out = [b22, zero, -b22, b21, b22, zero, b21 + b22] if b11 is None else _right(b11, b12, b21, b22)
    return [(7 * group + i, v) for i, v in enumerate(out)]


def _product576(mm):
    def group(b):
        x2, x3, x4, x5, xj, e12, e21 = [mm(7 * p + b, 7 * p + b, _ORDER.index(b)) for p in range(7)]
        return [[x4 - x5, (x3 + x5) + (xj + e12)], [(x2 + x4) + (xj + e21), x3 - x2]]

    def extra(r, c):
        xi, e11, e22 = [mm(49 + 2 * p + r, 49 + 2 * p + c, 0) for p in range(3)]
        return {(0, 0): xi + e11, (1, 1): xi + e22}

    return _collapse(group, extra)


def _left49(b, x):
    def inner(i, j):
        (r, c, _), *rest = _LEFT[b]
        v = x(2 * i + r, 2 * j + c)
        for r, c, sign in rest:
            v = v + x(2 * i + r, 2 * j + c) if sign > 0 else v - x(2 * i + r, 2 * j + c)
        return v
    return [(7 * a + b, v) for a, v in enumerate(_left(inner(0, 0), inner(0, 1), inner(1, 0), inner(1, 1)))]


def _right49(x):
    inner = [[_right(x[2 * i][2 * j], x[2 * i][2 * j + 1], x[2 * i + 1][2 * j], x[2 * i + 1][2 * j + 1])
              for j in range(2)] for i in range(2)]
    for b in (4, 6, 0, 1, 3, 2, 5):
        for a, v in enumerate(_right(inner[0][0][b], inner[0][1][b], inner[1][0][b], inner[1][1][b])):
            yield 7 * a + b, v


def _barrel(v):
    lane = _lane_id(v[0].shape[0])
    q = [v[(-p) % 4] for p in range(4)]
    q = [jnp.where((lane & 1) != 0, q[(p - 1) % 4], q[p]) for p in range(4)]
    return [jnp.where((lane & 2) != 0, q[(p - 2) % 4], q[p]) for p in range(4)]


def _split_phases(tiles):
    return _barrel([t if j == 0 else pltpu.roll(t, j, 1) for j, t in enumerate(tiles)])


def _merge_phases(phases):
    return [t if j == 0 else pltpu.roll(t, LANE - j, 1) for j, t in enumerate(_barrel(phases))]


def _dft4(u, sign):
    (r0, i0), (r1, i1), (r2, i2), (r3, i3) = u
    ar, ai, br, bi = r0 + r2, i0 + i2, r0 - r2, i0 - i2
    cr, ci, dr, di = r1 + r3, i1 + i3, r1 - r3, i1 - i3
    plus, minus = (br - di, bi + dr), (br + di, bi - dr)
    return [(ar + cr, ai + ci), plus if sign > 0 else minus, (ar - cr, ai - ci), minus if sign > 0 else plus]


def _make_kernel(cfg):
    def kernel(zero_ref, x_hbm, k_hbm, v_hbm, sk_hbm, ssm_hbm, sd_hbm, w1_hbm, w2_hbm, w3_hbm, w4_hbm, gw_hbm,
               wf_hbm, wi_hbm, out_hbm,
               k_v, v_v, sk_v, ssm_v, sd_v, w1_v, w2_v, w3_v, w4_v, gw_v, wf_v, wi_v, out_v, col_v, arena, sems,
               *buffers):
        x_v, shifted, normed, acc = [buffers[NUNIT * k:NUNIT * (k + 1)] for k in range(4)]
        square, hidden = buffers[4 * NUNIT:4 * NUNIT + 2], buffers[4 * NUNIT + 2:]

        copies = {}

        def copy(name, src, dst):
            copies[name] = pltpu.make_async_copy(src, dst, sems.at[len(copies)])

        def copy_x(u):
            copy(("x", u), x_hbm.at[:, pl.ds(u * UNIT, UNIT)], x_v[u])

        def copy_chunks(name, src, dst, first, last):
            cols = pl.ds(first * FCH, (last - first) * FCH)
            copy(name, src.at[:, cols], dst.at[:, cols])

        copy("gw", gw_hbm, gw_v)
        copy_x(0)
        copy("w1", w1_hbm, w1_v)
        for u in range(1, NUNIT):
            copy_x(u)
        copy("w2", w2_hbm, w2_v)
        copy_chunks("w3a", w3_hbm, w3_v, 0, FIRST[1])
        copy_chunks("w4a", w4_hbm, w4_v, 0, FIRST[1])
        copy_chunks("w3b", w3_hbm, w3_v, FIRST[1], NCH)
        copy_chunks("w4b", w4_hbm, w4_v, FIRST[1], NCH)
        copy("sk", sk_hbm, sk_v)
        copy("sd", sd_hbm, sd_v)
        copy("wf", wf_hbm, wf_v)
        copy("wi", wi_hbm, wi_v)
        copy("ssm", ssm_hbm, ssm_v.at[pl.ds(0, D)])
        copy("k", k_hbm, k_v.at[pl.ds(0, D)])
        copy("v", v_hbm, v_v)
        for c in copies.values():
            c.start()
        for first, last in zip((0,) + cfg["outs"], cfg["outs"]):
            cols = pl.ds(first * UNIT, (last - first) * UNIT)
            copy(("out", last), out_v.at[:, cols], out_hbm.at[:, cols])

        def wait(*names):
            for name in names:
                copies[name].wait()

        words = arena.bitcast(u32)
        zero = jnp.clip(zero_ref[0], 0, 1)
        val, jobs, recent = {}, [], []
        clock = dict(now=0.0, room=0.0, budget=0.0, cool=0.0, pinned=0.0, pending=False, slot=0)

        def tile(j):
            return slice(j * LANE, (j + 1) * LANE)

        def put(cell, x):
            arena[cell] = x.astype(bf16)

        def as_bf16(w):
            return pltpu.bitcast(w.reshape(w.shape[0] * ROW // 2, LANE), bf16)

        def seal(ref, back=None):
            early = cfg["early_back"] if clock["now"] < 23500 else 0
            due = clock["now"] - (back or cfg["back"]) - early
            mark = jnp.zeros((8, LANE), f32)
            for t, m, r in reversed(recent):
                if t <= due:
                    mark = m[r:r + 8, :LANE]
                    break
            view = ref if ref.dtype == f32 else ref.bitcast(f32)
            if len(ref.shape) == 2:
                view[pl.ds(pl.multiple_of(view.shape[0] - ROW + 8 * zero, 8), 8), 0:LANE] = mark
            elif ref.shape[1] > ROW:
                view[ref.shape[0] - 1, pl.ds(pl.multiple_of(8 * zero, 8), 8), :] = mark
            else:
                view[ref.shape[0] - 2 + zero] = mark

        def step(job):
            cost = next(job["steps"], None)
            if cost is None:
                jobs.remove(job)
            else:
                clock["budget"] -= cost
                job["left"] -= cost
                clock["pending"] = True

        def finish_jobs(names):
            for job in [j for j in jobs if j["name"] in names]:
                while job in jobs:
                    step(job)
            clock["budget"] = max(clock["budget"], 0.0)

        def tick(cycles, weight, calm=True):
            hot = min(cycles, max(clock["cool"], 0.0))
            clock["cool"] -= cycles
            clock["now"] += cycles
            room = weight * (cycles - hot)
            rate, work = cfg["rate"], 0
            for job in sorted(jobs, key=lambda j: j["due"]):
                work += job["left"]
                rate = max(rate, work / max(room_before[job["due"][0]] - clock["room"] - cfg["margin"], 1.0))
            clock["room"] += room
            clock["budget"] = min(clock["budget"] + min(rate, cfg["max_rate"]) * room, 30.0)
            while clock["budget"] > 0:
                ready = [j for j in jobs if (calm and clock["cool"] < 0) or j["name"][0] != "conv_mul"]
                if not ready:
                    break
                step(min(ready, key=lambda j: j["due"]))

        def mm(lhs, rhs, weight, width=1, calm=True, turn=False):
            n, start = lhs[0][1], clock["now"]
            cycles = ROW * len(lhs) * width / 4
            pinned = {}
            for j in range(n):
                tick(cycles, weight, calm)
                if clock["pending"] and clock["now"] >= clock["pinned"] + cfg["gap"]:
                    k = j % len(lhs)
                    pinned[k, j] = words[pl.ds(lhs[k][0] + j + zero, 1)]
                    clock["pinned"], clock["pending"] = clock["now"], False
            tiles = []
            for k, (cell, _) in enumerate(lhs):
                parts, j0 = [], 0
                for j in sorted(j for t, j in pinned if t == k):
                    parts += [words[cell + j0:cell + j]] if j > j0 else []
                    parts.append(pinned[k, j])
                    j0 = j + 1
                parts += [words[cell + j0:cell + n]] if n > j0 else []
                tiles.append(as_bf16(parts[0] if len(parts) == 1 else jnp.concatenate(parts, axis=0)))
            a = tiles[0] if len(tiles) == 1 else jnp.concatenate(tiles, axis=1)
            m = jax.lax.dot_general(a, rhs(), (((1,), (int(turn),)), ((), ())), preferred_element_type=f32)
            recent.extend((start + j * cycles, m, j * ROW) for j in range(n))
            return m

        def up_cell(c, i):
            return _BASE["weights"] + _WEIGHTS * c + 8 * i

        def down_cell(c, i):
            return up_cell(c, 55) + 9 * i

        def prep_square(src, which):
            tail = src[4 * LANE:D, :]
            tiles = [src[k * LANE:(k + 1) * LANE, :] for k in range(4)] + [jnp.concatenate([tail, tail], axis=0)]
            for k, t in enumerate(tiles):
                square[which][D // 2 * k:D // 2 * (k + 1)] = pltpu.bitcast(t.T, u32)

        def prep_up(c):
            for r in range(0, LANE, ROW):
                for group in range(9):
                    for i, x in _right576(group, r, lambda j, k: w3_v[k:k + ROW, tile(4 * c + j)].astype(f32)):
                        put(up_cell(c, i) + r // ROW, x)
                    yield 36

        def prep_down(c):
            for r in range(0, QD, ROW):
                for b in _ORDER:
                    for i, x in _left49(b, lambda i, j: w4_v[
                            i * QD + r:i * QD + r + ROW, tile(4 * c + (j ^ 1))].astype(f32)):
                        put(down_cell(c, i) + r // ROW, x)
                    yield 40

        def columns(which):
            for j in which:
                row = sk_v[...].astype(f32)[j:j + 1] if j < 4 else (sd_v, gw_v)[j - 4][...].astype(f32).reshape(1, D)
                col_v[j] = jnp.broadcast_to(row, (LANE, D)).T

        def x_rows(u, j, r, n=ROW):
            return x_v[u][r:r + n, tile(j)].astype(f32)

        def prep_x(u):
            stats = []
            for slot, cost in enumerate((270, 230)):
                total = None
                for r in range(0, D, ROW):
                    term = [jnp.square(x_rows(u, j, r) - stats[0][j]) if stats else x_rows(u, j, r) for j in range(4)]
                    if not stats:
                        if r % QD == 0:
                            seal(col_v, cfg["lane_back"] - 100)
                        term += [t * col_v[5, r:r + ROW] for t in term]
                    total = term if total is None else [a + t for a, t in zip(total, term)]
                    if (r + ROW) % QD == 0:
                        for k in range(0, len(total), 4):
                            put(_BASE["sums"] + slot + k, (total[k] + total[k + 1]) + (total[k + 2] + total[k + 3]))
                        yield cost
                sums = [jnp.sum(a, axis=0, keepdims=True) for a in total]
                stats.append([a * (1.0 / D) for a in sums[:4]])
                for j, logit in enumerate(sums[4:]):
                    g = jax.nn.sigmoid(logit)
                    val["gate", 4 * u + j] = g
                    val["rest", 4 * u + j] = 1.0 - g
                    val["out", 4 * u + j] = (1.0 - g) * GELU_OUT
            scale = [jax.lax.rsqrt(v + LN_EPS) * GELU_IN for v in stats[1]]
            shift = [m * s for m, s in zip(stats[0], scale)]
            for r in range(0, D, ROW):
                for j in range(4):
                    put(_BASE["x"] + DC * (4 * (u % 2) + j) + r // ROW, x_rows(u, j, r) * scale[j] - shift[j])
                yield 28

        def square_product(which, source, cell):
            lhs, out = square[which], [[None] * 4 for _ in range(4)]
            for j in range(4):
                for i in range(4):
                    a = pltpu.bitcast(jnp.concatenate(
                        [lhs[(D * k + QD * i) // 2:(D * k + QD * (i + 1)) // 2] for k in range(5)], axis=1), bf16)
                    start, parts = clock["now"], []
                    for k in range(0, DC, 6):
                        tick(5 * QD / 4 / 6, cfg["room_square"])
                        first = cell + DC * j + k
                        if clock["pending"] and source is words:
                            parts += [words[pl.ds(first + zero, 1)], words[first + 1:first + 6]]
                            clock["pending"] = False
                        else:
                            parts.append(source[first:first + 6])
                    m = jnp.dot(a[:, :D], as_bf16(jnp.concatenate(parts, axis=0)), preferred_element_type=f32)
                    recent.extend((start + r * 5 / 4, m, r) for r in range(0, QD, ROW))
                    out[i][j] = m
            return out

        def mix_in(u):
            seal(arena)
            h = square_product(0, words, _BASE["x"] + 4 * DC * (u % 2))
            lane = _lane_id(QD)

            def keep(u, j, i, x):
                shifted[u][DC * j + 9 * i:DC * j + 9 * (i + 1)] = x.astype(bf16).reshape(9, ROW, LANE)

            for i, n in enumerate(SHIFTS):
                rolled = [pltpu.roll(_gelu2(z), n % LANE, 1) for z in h[i]]
                if n > 0:
                    for j in range(4):
                        before = rolled[j - 1] if j else val.get(("edge", i), 0.0)
                        keep(u, j, i, jnp.where(lane >= n, rolled[j], before))
                else:
                    if u > 0:
                        keep(u - 1, 3, i, jnp.where(lane < LANE + n, val["edge", i], rolled[0]))
                    for j in range(3 if u < NUNIT - 1 else 4):
                        keep(u, j, i, jnp.where(lane < LANE + n, rolled[j], rolled[j + 1] if j < 3 else 0.0))
                val["edge", i] = rolled[3]

        def mix_out(u):
            seal(arena)
            seal(shifted[u])
            y = square_product(1, shifted[u].bitcast(u32), 0)
            for j in range(4):
                x1, first, second = [], None, None
                for r in range(0, D, ROW):
                    i, k = divmod(r, QD)
                    x1.append(x_rows(u, j, r) + GELU_OUT * y[i][j][k:k + ROW])
                    pilot = x1[0][:1] if r == 0 else pilot
                    d = x1[-1] - pilot
                    first = d if first is None else first + d
                    second = d * d if second is None else second + d * d
                offset = jnp.sum(first, axis=0, keepdims=True) * (1.0 / D)
                var = jnp.maximum(jnp.sum(second, axis=0, keepdims=True) * (1.0 / D) - offset * offset, 0.0)
                scale = jax.lax.rsqrt(var + LN_EPS) * GELU_IN
                shift = (pilot + offset) * scale
                normal = [z * scale - shift for z in x1]
                for r, z in enumerate(x1):
                    val["skip", 4 * u + j, r] = val["rest", 4 * u + j] * z
                for k in range(5):
                    rows = normal[8 * k:8 * k + 8] if k < 4 else normal[32:] * 2
                    normed[u][5 * j + k] = jnp.concatenate(rows, axis=0).T

        def token_cell(u, i):
            return _BASE["tokens"] + 8 * (55 * u + i)

        def prep_tokens(u):
            for r in range(0, LANE, ROW):
                for group in range(9):
                    if group % 3 == 0:
                        seal(normed[u])
                    for i, x in _left576(group, lambda i, k: normed[u][5 * i + k, r:r + ROW]):
                        put(token_cell(u, i) + r // ROW, x)
                    yield 30

        def up(n, s, u, c, r):
            h = _product576(lambda a, b, k: mm([(token_cell(u, a) + r // ROW, PIECE // ROW)],
                                               lambda: as_bf16(words[up_cell(c, b):up_cell(c, b) + 8]),
                                               cfg["room_up"][k], calm=False))
            g = [[_gelu2(h[j][i ^ 1]) for j in range(4)] for i in range(4)]
            for k in range(0, PIECE, ROW):
                for p, x in _right49([[z[k:k + ROW] for z in row] for row in g]):
                    hidden[n % 2][8 * (49 * (c - FIRST[s]) + p) + (r + k) // ROW] = x.astype(bf16)
            clock["cool"] = cfg["cool"] * PIECE / 64

        def down(n, s, u, p):
            chunks = range(FIRST[s], FIRST[s + 1])
            source = hidden[n % 2].bitcast(u32)
            if p == 0:
                seal(source)
                if s > 0:
                    seal(acc[u])
            m = mm([(down_cell(c, p), 9) for c in chunks],
                   lambda: jnp.concatenate([as_bf16(source[8 * (49 * k + p):8 * (49 * k + p + 1)])
                                            for k in range(len(chunks))], axis=1), cfg["room_down"], turn=True)
            if s > 0:
                m = m + acc[u][p]
            if FIRST[s + 1] == NCH:
                val["acc", u, p] = m
            else:
                acc[u][p] = m

        def finish(u):
            for r in range(0, QD, ROW):
                y = _collapse(lambda b: _result([val["acc", u, 7 * a + b][r:r + ROW] for a in range(7)]))
                for i in range(4):
                    for j in range(4):
                        t, row = 4 * u + j, i * QD + r
                        base = jnp.concatenate([val["base", t, row], val["base", t, row + 8]], axis=0)
                        out_v[row:row + ROW, tile(t)] = (base + val["out", t] * y[i][j]).astype(bf16)
            if u + 1 in cfg["outs"]:
                copies["out", u + 1].start()

        def conv_cell(n, kind, rho):
            return _BASE["conv"] + 64 * (n % _RING) + 16 * kind + 4 * rho

        def conv_inputs(n):
            rows = slice(n * ROW, (n + 1) * ROW)
            lane = _lane_id(ROW // 2)
            seal(col_v, cfg["lane_back"])
            col = [col_v[j, rows] for j in range(4)]
            prev = [jnp.zeros((ROW // 2, LANE), u32)] * 3
            for i in range(NUNIT):
                seal(ssm_v, cfg["lane_back"])
                taps = _split_phases([pltpu.bitcast(ssm_v[rows, tile(4 * i + j)], u32) for j in range(4)])
                for rho in range(4):
                    words[conv_cell(n, 0, rho) + i] = taps[rho]
                yield 16
                seal(k_v, cfg["lane_back"])
                kv = []
                for t in range(4 * i, 4 * i + 4):
                    key = k_v[rows, tile(t)]
                    rolled = [pltpu.roll(pltpu.bitcast(key, u32), j, 1) for j in (1, 2, 3)]
                    total = key.astype(f32) * col[0]
                    for j in (1, 2, 3):
                        late = jnp.where(lane >= j, rolled[j - 1], prev[j - 1])
                        total = total + pltpu.bitcast(late, bf16).astype(f32) * col[j]
                    prev = rolled
                    kv.append(total * v_v[rows, tile(t)].astype(f32))
                    if t % 4 == 1:
                        yield 60
                for rho, x in enumerate(_split_phases(kv)):
                    put(conv_cell(n, 1, rho) + i, x)
                yield 80

        def conv_forward(n, kind):
            seal(arena)
            last = None
            for i in range(0, NUNIT, 2):
                u = {rho: mm([(conv_cell(n, kind, rho) + i, 2)], lambda: pltpu.bitcast(wf_v[rho], bf16),
                             cfg["room_conv"], 2) for rho in (0, 2, 1, 3)}
                for k in range(2):
                    rows = slice(k * ROW, (k + 1) * ROW)
                    z = [(u[rho][rows, :LANE], u[rho][rows, LANE:]) for rho in range(4)]
                    if kind == 0:
                        if last is None:
                            z[0] = (z[0][0] + col_v[4, n * ROW:(n + 1) * ROW], z[0][1])
                        z, last = z if last is None else [(a[0] - b[1], a[1] + b[0]) for a, b in zip(z, last)], z
                    val["spectrum", n, kind, i + k] = _dft4(z, -1)

        pairs = ((0, 3), (1, 2))

        def conv_multiply(n):
            for r in range(0, ROW, 8):
                def product(i, s):
                    re = im = None
                    for j in range(i + 1):
                        xr, xi = [z[r:r + 8] for z in val["spectrum", n, 1, j][s]]
                        kr, ki = [z[r:r + 8] for z in val["spectrum", n, 0, i - j][s]]
                        re = (xr * kr if re is None else re + xr * kr) - xi * ki
                        im = (xr * ki if im is None else im + xr * ki) + xi * kr
                    return re, im

                for h, pair in enumerate(pairs):
                    a, b = [_dft4([product(i, s) for s in range(4)], 1) for i in pair]
                    for rho in range(4):
                        for part in range(2):
                            put(conv_cell(n, 2 + part, rho) + r // 4 + h,
                                jnp.concatenate([a[rho][part], b[rho][part]], axis=0))
                    yield 185

        def conv_inverse(n):
            seal(arena)
            for k in range(2):
                ys = [mm([(conv_cell(n, 2 + part, rho) + 2 * k, 2) for part in range(2)],
                         lambda: pltpu.bitcast(wi_v[rho], bf16), cfg["room_conv"]) for rho in range(4)]
                row = n * ROW + 8 * k
                for q, i in enumerate(pairs[0] + pairs[1]):
                    y = _merge_phases([m[8 * q:8 * q + 8] for m in ys])
                    for j in range(4):
                        t = 4 * i + j
                        val["base", t, row] = ((val["gate", t] * y[j]) * x_rows(i, j, row, 8)
                                               + val["skip", t, n][8 * k:8 * k + 8])

        def job(kind, i):
            make = dict(x=prep_x, tokens=prep_tokens, up=prep_up, down=prep_down,
                        conv_in=conv_inputs, conv_mul=conv_multiply)[kind]
            return (kind, i), lambda: make(i)

        room = cfg["room_square"] * 20 * QD

        def first_stage(u, *frees):
            return lambda: mix_in(u), [("x", u)], frees, room

        def second_stage(u):
            return lambda: mix_out(u), (), [job("tokens", u)], room

        stream = [
            (lambda: wait("gw"), (), (), 0),
            (lambda: columns((5,)), (), (), 0),
            (lambda: wait(("x", 0)), (), [job("x", 0)], 0),
            (lambda: wait("w1"), [("x", 0)], (), 0),
            (lambda: prep_square(w1_v, 0), (), (), 0),
            (lambda: wait(("x", 1)), (), [job("x", 1)], 0),
            first_stage(0),
            (lambda: wait(("x", 2), ("x", 3)), (), [job("x", 2)], 0),
            first_stage(1, job("x", 3)),
            first_stage(2),
            (lambda: (wait("w2", "w3a"), prep_square(w2_v, 1)), (), [job("up", c) for c in range(FIRST[1])], 0),
            first_stage(3),
            second_stage(0),
            second_stage(1),
            second_stage(2),
            second_stage(3),
        ]

        stream.insert(cfg["down_ready"], (lambda: wait("w4a"), (), [job("down", c) for c in range(FIRST[1])], 0))
        slots = [(s, u) for s in range(len(FIRST) - 1) for u in range(NUNIT)]
        plan, begin = [], []
        for n, (s, u) in enumerate(slots):
            begin.append(len(plan))
            for c in range(FIRST[s], FIRST[s + 1]):
                for r in range(0, LANE, PIECE):
                    plan.append((len(plan) + 0.25, (
                        lambda n=n, s=s, u=u, c=c, r=r: up(n, s, u, c, r), [("up", c), ("tokens", u)], (),
                        (12 * cfg["room_up"][0] + 7 * sum(cfg["room_up"])) * PIECE / 4 - cfg["cool"] * PIECE / 64)))
        begin += [len(plan), len(plan) + 1]
        for n, (s, u) in enumerate(slots):
            count = begin[n + 2] - begin[n + 1]
            for k, p in enumerate(7 * a + b for b in _ORDER for a in range(7)):
                plan.append((begin[n + 1] + (k * count) // 49 + 0.5 + 0.3 * ((k * count) % 49) / 49, (
                    lambda n=n, s=s, u=u, p=p: down(n, s, u, p),
                    [("down", c) for c in range(FIRST[s], FIRST[s + 1])] if k == 0 else (), (),
                    cfg["room_down"] * (FIRST[s + 1] - FIRST[s]) * QD / 4)))
            if FIRST[s + 1] == NCH:
                plan.append((begin[n + 2] - 0.2, (lambda u=u: finish(u), (), (), 0)))
        plan.append((cfg["late"] + 0.1, (
            lambda: (wait("w3b", "w4b", "sk", "sd", "wf", "wi", "ssm", "k", "v"), columns(range(5))), (),
            [job(kind, c) for c in range(FIRST[1], NCH) for kind in ("up", "down")]
            + [job("conv_in", n) for n in range(2)], 0)))
        for n in range(NCONV):
            pos = round(cfg["conv"][0] + (cfg["conv"][1] - cfg["conv"][0]) * n / NCONV)
            room = cfg["room_conv"] * 8 * ROW
            frees = [job("conv_mul", n)] + [job("conv_in", m) for m in (n + 2,) if m < NCONV]
            plan += [(pos + 0.9, (lambda n=n: conv_forward(n, 0), [("conv_in", n)], (), room)),
                     (pos + 0.91, (lambda n=n: conv_forward(n, 1), (), frees, room)),
                     (pos + cfg["lag"] + 0.7, (lambda n=n: conv_inverse(n), [("conv_mul", n)], (), room))]
        plan.sort(key=lambda e: e[0])
        stream += [e[1] for e in plan]

        due, room_before = {}, [0.0]
        for k, (_, needs, _, room) in enumerate(stream):
            room_before.append(room_before[-1] + room)
            for name in needs:
                due.setdefault(name, k)
        for name in due:
            if name[0] in ("up", "down"):
                due[name] = min(due[name], due["conv_in", 0])
        for k, (task, needs, frees, _) in enumerate(stream):
            clock["room"] = room_before[k]
            finish_jobs(needs)
            task()
            for name, make in frees:
                jobs.append(dict(name=name, steps=make(), due=(due[name], len(jobs)), left=WORK[name[0]]))
        wait(*[("out", last) for last in cfg["outs"]])

    return kernel


def make_fn(cfg):
    def fn(A_q, A_k, A_v, A_shift_k, A_ssm_k, A_ssm_D, B_x, B_w1, B_w2, B_w3, B_w4, gate_w):
        del B_x

        def feature_major(a):
            return jnp.swapaxes(a, 1, 2).reshape(D, S)

        args = (feature_major(A_q), feature_major(A_k), feature_major(A_v), A_shift_k.T, A_ssm_k, A_ssm_D,
                B_w1, B_w2, B_w3, B_w4.T, gate_w, jnp.asarray(_WF), jnp.asarray(_WI))
        plain = pltpu.VMEM((D, S), bf16)
        marked = pltpu.VMEM((D + 2 * ROW, S), bf16)
        out = pl.pallas_call(
            _make_kernel(cfg),
            out_shape=jax.ShapeDtypeStruct((D, S), bf16),
            in_specs=[pl.BlockSpec(memory_space=pltpu.SMEM)] + [pl.BlockSpec(memory_space=pl.ANY)] * len(args),
            out_specs=pl.BlockSpec(memory_space=pl.ANY),
            scratch_shapes=[
                marked, plain, pltpu.VMEM((4, D), bf16), marked, pltpu.VMEM((D,), bf16),
                pltpu.VMEM((D, D), bf16), pltpu.VMEM((D, D), bf16),
                pltpu.VMEM((D, F), bf16), pltpu.VMEM((D, F), bf16), pltpu.VMEM((D,), bf16),
                pltpu.VMEM(_WF.shape, u32), pltpu.VMEM(_WI.shape, u32), plain,
                pltpu.VMEM((6 + 1, D, LANE), f32),
                pltpu.VMEM((_NCELL, ROW, LANE), bf16),
                pltpu.SemaphoreType.DMA((14 + NUNIT + len(cfg["outs"]),)),
                *[pltpu.VMEM((D, UNIT), bf16)] * NUNIT,
                *[pltpu.VMEM((4 * DC + 2, ROW, LANE), bf16)] * NUNIT,
                *[pltpu.VMEM((20 + 1, LANE, LANE), f32)] * NUNIT,
                *[pltpu.VMEM((49 + 1, QD, LANE), f32)] * NUNIT,
                *[pltpu.VMEM((5 * D // 2, LANE), u32)] * 2,
                *[pltpu.VMEM((4 * 49 * 8 + 2, ROW, LANE), bf16)] * 2,
            ],
            compiler_params=pltpu.CompilerParams(vmem_limit_bytes=127 * 1024 * 1024),
            name="mlp_gated_mix",
        )(jnp.asarray(np.zeros((1,), np.int32)), *args)
        return jnp.swapaxes(out.reshape(1, D, S), 1, 2)
    return fn


@jax.jit
def pallas_gated_mix__ssm_conv_h3__mixer_s_mlp__prompt_kernel(
    A_q, A_k, A_v, A_shift_k, A_ssm_k, A_ssm_D, B_x, B_w1, B_w2, B_w3, B_w4, gate_w,
):
    return make_fn(CFG)(A_q, A_k, A_v, A_shift_k, A_ssm_k, A_ssm_D, B_x, B_w1, B_w2, B_w3, B_w4, gate_w)
```

```python
import math

import jax
import jax.numpy as jnp
import numpy as np
import jax.experimental.pallas as pl
import jax.experimental.pallas.tpu as pltpu

D, S, F = 576, 2048, 4608
LANE = 128
ROW = 16
DC = D // ROW
UNIT = 4 * LANE
NUNIT = S // UNIT
QD = D // 4
FCH = 4 * LANE
NCH = F // FCH
FIRST = (0, 4, 8, 9)
PIECE = 32
NCONV = D // ROW
SHIFTS = (1, -1, 2, -2)
TILE_OF = (0, 2, 1, 3)
LN_EPS = 1e-5

f32, bf16, u32 = jnp.float32, jnp.bfloat16, jnp.uint32

_C0 = math.sqrt(2.0 / math.pi)
GELU_IN = (_C0 * 0.044715) ** (1.0 / 3.0)
GELU_A = _C0 / GELU_IN
GELU_OUT = 0.5 / GELU_IN

CFG = dict(
    back=180, early_back=200, lane_back=450, gap=45,
    rate=1.0, max_rate=2.5, margin=150, cool=150,
    room_up=(1, 1, 1, 0.8, 0.8, 0.6, 0.6), room_down=1.0, room_conv=0.5, room_square=1.1,
    late=24, conv=(54, 126), lag=2.7,
    outs=(4, 6, 7, 8),
)
WORK = dict(up=2592, down=2520, x=3000, tokens=2160, conv_in=624, conv_mul=740)

_WEIGHTS = 55 * 8 + 49 * 9
_RING = 3
_SIZES = dict(weights=NCH * _WEIGHTS, tokens=NUNIT * 55 * 8, conv=_RING * 64, sums=8, head=4, spare=2)
_BASE = dict(zip(_SIZES, np.cumsum([0] + list(_SIZES.values())).tolist()))
_BASE["x"] = _BASE["weights"] + FIRST[1] * _WEIGHTS
_NCELL = sum(_SIZES.values())


def _dft_tables():
    lane = np.arange(LANE)
    fwd = []
    for rho in range(4):
        j = (lane - rho) % 4
        t = LANE * j + (lane - j) % LANE
        theta = 2.0 * np.pi * np.outer(t, 2.0 * lane + 0.5) / (2 * UNIT)
        fwd.append(np.concatenate([np.cos(theta), -np.sin(theta)], axis=1))
    fwd = np.stack(fwd)
    inv = fwd.transpose(0, 2, 1) / UNIT

    def words(a):
        half = np.ascontiguousarray(a.astype(np.float32).astype(bf16)).view(np.uint16).astype(np.uint32)
        return half[:, 0::2] | (half[:, 1::2] << 16)
    return words(fwd), words(inv)


_WF, _WI = _dft_tables()


def _gelu2(z):
    return z + z * jnp.tanh(z * (z * z + GELU_A))


def _lane_id(rows):
    return jax.lax.broadcasted_iota(jnp.int32, (rows, LANE), 1)


def _left(a11, a12, a21, a22):
    return [a11 + a22, a21 + a22, a11, a22, a11 + a12, a21 - a11, a12 - a22]


def _right(b11, b12, b21, b22):
    return [b11 + b22, b11, b12 - b22, b21 - b11, b22, b11 + b12, b21 + b22]


def _result(m):
    return [[m[0] + m[3] - m[4] + m[6], m[2] + m[4]],
            [m[1] + m[3], m[0] - m[1] + m[2] + m[5]]]


_LEFT = (((0, 0, 1), (1, 1, 1)), ((1, 0, 1), (1, 1, 1)), ((0, 0, 1),), ((1, 1, 1),), ((0, 0, 1), (0, 1, 1)),
         ((1, 0, 1), (0, 0, -1)), ((0, 1, 1), (1, 1, -1)))
_ORDER = (0, 6, 3, 4, 1, 2, 5)


def _collapse(group, extra):
    out = [[None] * 4 for _ in range(4)]

    def plus(z, r, c):
        add = extra(r, c)
        return [[z[i][j] + add[i, j] if (i, j) in add else z[i][j] for j in range(2)] for i in range(2)]

    def both(fn, a, b):
        return [[fn(a[i][j], b[i][j]) for j in range(2)] for i in range(2)]

    def emit(z, r, c):
        for i in range(2):
            for j in range(2):
                out[2 * i + r][2 * j + c] = z[i][j]

    y0 = group(0)
    first = both(jnp.add, plus(y0, 0, 0), group(6))
    y3 = group(3)
    first = both(jnp.add, first, y3)
    y4 = group(4)
    emit(both(jnp.subtract, first, y4), 0, 0)
    low = plus(y3, 1, 0)
    y1 = group(1)
    emit(both(jnp.add, low, y1), 1, 0)
    last = both(jnp.subtract, y0, y1)
    high = plus(y4, 0, 1)
    y2 = group(2)
    emit(both(jnp.add, high, y2), 0, 1)
    last = plus(both(jnp.add, last, y2), 1, 1)
    emit(both(jnp.add, last, group(5)), 1, 1)
    return out


def _left576(group, t):
    lo = _lane_id(ROW) < LANE // 2
    if group >= 7:
        r = group - 7
        u0, u2, v0, v2 = t(r, 0), t(r, 2), t(2 + r, 0), t(2 + r, 2)
        return [(49 + r, u0 + v2), (51 + r, jnp.where(lo, u2 - v2, t(r, 4))),
                (53 + r, jnp.where(lo, v0 - u0, t(2 + r, 4)))]
    pair = (lambda u, v: (v(0) + v(2), v(1) + v(3)),
            lambda u, v: (jnp.where(lo, u(0), v(2)), v(3)),
            lambda u, v: (jnp.where(lo, v(2), u(0)), u(1)),
            lambda u, v: (u(0) + u(2), u(1) + u(3)),
            lambda u, v: (jnp.where(lo, 0.0, u(0) + v(2)), u(1) + v(3)),
            lambda u, v: (jnp.where(lo, u(4), u(2) - v(2)), u(3) - v(3)),
            lambda u, v: (jnp.where(lo, v(4), v(0) - u(0)), v(1) - u(1)))[group]
    top, bottom = [pair(lambda k: t(r, k), lambda k: t(2 + r, k)) for r in range(2)]
    return [(7 * group + i, x) for i, x in enumerate(_left(*top, *bottom))]


def _right576(group, r, x):
    zero = jnp.zeros((ROW, LANE), f32)
    if group >= 7:
        c = group - 7
        if r >= 64:
            return [(49 + c, zero), (51 + c, x(c, 448 + r)), (53 + c, x(2 + c, 448 + r))]
        p1, q2 = x(c, r), x(2 + c, 256 + r)
        return [(49 + c, p1 + q2), (51 + c, x(c, 256 + r) + q2), (53 + c, p1 + x(2 + c, r))]

    def part(c, k):
        p1, p2, ps = [lambda d=d: x(c, d + k) for d in (0, 256, 512)]
        q1, q2, qs = [lambda d=d: x(2 + c, d + k) for d in (0, 256, 512)]
        if k < 64:
            return (p1, lambda: q1() - q2(), lambda: p2() - p1(), q2, lambda: None, qs, ps)[group]()
        return (lambda: -q1(), lambda: q2() - q1(), lambda: p1() - p2(), lambda: -p2(), lambda: q1() + p2(),
                lambda: p2() + q2(), lambda: p1() + q1())[group]()

    b11, b12, b21, b22 = part(0, r), part(1, r), part(0, LANE + r), part(1, LANE + r)
    out = [b22, zero, -b22, b21, b22, zero, b21 + b22] if b11 is None else _right(b11, b12, b21, b22)
    return [(7 * group + i, v) for i, v in enumerate(out)]


def _product576(mm):
    def group(b):
        x2, x3, x4, x5, xj, e12, e21 = [mm(7 * p + b, 7 * p + b, _ORDER.index(b)) for p in range(7)]
        return [[x4 - x5, (x3 + x5) + (xj + e12)], [(x2 + x4) + (xj + e21), x3 - x2]]

    def extra(r, c):
        xi, e11, e22 = [mm(49 + 2 * p + r, 49 + 2 * p + c, 0) for p in range(3)]
        return {(0, 0): xi + e11, (1, 1): xi + e22}

    return _collapse(group, extra)


def _left49(b, x):
    def inner(i, j):
        (r, c, _), *rest = _LEFT[b]
        v = x(2 * i + r, 2 * j + c)
        for r, c, sign in rest:
            v = v + x(2 * i + r, 2 * j + c) if sign > 0 else v - x(2 * i + r, 2 * j + c)
        return v
    return [(7 * a + b, v) for a, v in enumerate(_left(inner(0, 0), inner(0, 1), inner(1, 0), inner(1, 1)))]


def _right49(x):
    inner = [[_right(x[2 * i][2 * j], x[2 * i][2 * j + 1], x[2 * i + 1][2 * j], x[2 * i + 1][2 * j + 1])
              for j in range(2)] for i in range(2)]
    for b in (4, 6, 0, 1, 3, 2, 5):
        for a, v in enumerate(_right(inner[0][0][b], inner[0][1][b], inner[1][0][b], inner[1][1][b])):
            yield 7 * a + b, v


def _barrel(v):
    lane = _lane_id(v[0].shape[0])
    q = [v[(-p) % 4] for p in range(4)]
    q = [jnp.where((lane & 1) != 0, q[(p - 1) % 4], q[p]) for p in range(4)]
    return [jnp.where((lane & 2) != 0, q[(p - 2) % 4], q[p]) for p in range(4)]


def _split_phases(tiles):
    return _barrel([t if j == 0 else pltpu.roll(t, j, 1) for j, t in enumerate(tiles)])


def _merge_phases(phases):
    return [t if j == 0 else pltpu.roll(t, LANE - j, 1) for j, t in enumerate(_barrel(phases))]


def _dft4(u, sign):
    (r0, i0), (r1, i1), (r2, i2), (r3, i3) = u
    ar, ai, br, bi = r0 + r2, i0 + i2, r0 - r2, i0 - i2
    cr, ci, dr, di = r1 + r3, i1 + i3, r1 - r3, i1 - i3
    plus, minus = (br - di, bi + dr), (br + di, bi - dr)
    return [(ar + cr, ai + ci), plus if sign > 0 else minus, (ar - cr, ai - ci), minus if sign > 0 else plus]


def _make_kernel(cfg):
    def kernel(zero_ref, x_hbm, k_hbm, v_hbm, sk_hbm, ssm_hbm, sd_hbm, w1_hbm, w2_hbm, w3_hbm, w4_hbm, gw_hbm,
               wf_hbm, wi_hbm, out_hbm,
               k_v, v_v, sk_v, ssm_v, sd_v, w1_v, w2_v, w3_v, w4_v, gw_v, wf_v, wi_v, out_v, col_v, arena, sems,
               *buffers):
        x_v, shifted, normed, acc = [buffers[NUNIT * k:NUNIT * (k + 1)] for k in range(4)]
        square, hidden = buffers[4 * NUNIT:4 * NUNIT + 2], buffers[4 * NUNIT + 2:]

        copies = {}

        def copy(name, src, dst):
            copies[name] = pltpu.make_async_copy(src, dst, sems.at[len(copies)])

        def copy_x(u):
            copy(("x", u), x_hbm.at[:, pl.ds(u * UNIT, UNIT)], x_v[u])

        def copy_chunks(name, src, dst, first, last):
            cols = pl.ds(first * FCH, (last - first) * FCH)
            copy(name, src.at[:, cols], dst.at[:, cols])

        copy("gw", gw_hbm, gw_v)
        copy_x(0)
        copy("w1", w1_hbm, w1_v)
        for u in range(1, NUNIT):
            copy_x(u)
        copy("w2", w2_hbm, w2_v)
        copy_chunks("w3a", w3_hbm, w3_v, 0, FIRST[1])
        copy_chunks("w4a", w4_hbm, w4_v, 0, FIRST[1])
        copy_chunks("w3b", w3_hbm, w3_v, FIRST[1], NCH)
        copy_chunks("w4b", w4_hbm, w4_v, FIRST[1], NCH)
        copy("sk", sk_hbm, sk_v)
        copy("sd", sd_hbm, sd_v)
        copy("wf", wf_hbm, wf_v)
        copy("wi", wi_hbm, wi_v)
        copy("ssm", ssm_hbm, ssm_v.at[pl.ds(0, D)])
        copy("k", k_hbm, k_v.at[pl.ds(0, D)])
        copy("v", v_hbm, v_v)
        for c in copies.values():
            c.start()
        for first, last in zip((0,) + cfg["outs"], cfg["outs"]):
            cols = pl.ds(first * UNIT // 2, (last - first) * UNIT // 2)
            copy(("out", last), out_v.at[:, cols], out_hbm.at[:, cols])

        def wait(*names):
            for name in names:
                copies[name].wait()

        words = arena.bitcast(u32)
        zero = jnp.clip(zero_ref[0], 0, 1)
        val, jobs, recent = {}, [], []
        clock = dict(now=0.0, room=0.0, budget=0.0, cool=0.0, pinned=0.0, pending=False)

        def tile(j):
            return slice(j * LANE, (j + 1) * LANE)

        def put(cell, x):
            arena[cell] = x.astype(bf16)

        def as_bf16(w):
            return pltpu.bitcast(w.reshape(w.shape[0] * ROW // 2, LANE), bf16)

        def seal(ref, back=None):
            early = cfg["early_back"] if clock["now"] < 2 * NUNIT * 20 * QD + 460 else 0
            due = clock["now"] - (back or cfg["back"]) - early
            mark = jnp.zeros((8, LANE), f32)
            for t, m, r in reversed(recent):
                if t <= due:
                    mark = m[r:r + 8, :LANE]
                    break
            view = ref if ref.dtype == f32 else ref.bitcast(f32)
            if len(ref.shape) == 2:
                view[pl.ds(pl.multiple_of(view.shape[0] - ROW + 8 * zero, 8), 8), 0:LANE] = mark
            elif ref.shape[1] > ROW:
                view[ref.shape[0] - 1, pl.ds(pl.multiple_of(8 * zero, 8), 8), :] = mark
            else:
                view[ref.shape[0] - 2 + zero] = mark

        def step(job):
            cost = next(job["steps"], None)
            if cost is None:
                jobs.remove(job)
            else:
                clock["budget"] -= cost
                job["left"] -= cost
                clock["pending"] = True

        def finish_jobs(names):
            for job in [j for j in jobs if j["name"] in names]:
                while job in jobs:
                    step(job)
            clock["budget"] = max(clock["budget"], 0.0)

        def tick(cycles, weight, calm=True):
            hot = min(cycles, max(clock["cool"], 0.0))
            clock["cool"] -= cycles
            clock["now"] += cycles
            room = weight * (cycles - hot)
            rate, work = cfg["rate"], 0
            for job in sorted(jobs, key=lambda j: j["due"]):
                work += job["left"]
                rate = max(rate, work / max(room_before[job["due"][0]] - clock["room"] - cfg["margin"], 1.0))
            clock["room"] += room
            clock["budget"] = min(clock["budget"] + min(rate, cfg["max_rate"]) * room, 30.0)
            while clock["budget"] > 0:
                ready = [j for j in jobs if (calm and clock["cool"] < 0) or j["name"][0] != "conv_mul"]
                if not ready:
                    break
                step(min(ready, key=lambda j: j["due"]))

        def mm(lhs, rhs, weight, width=1, calm=True, turn=False):
            n, start = lhs[0][1], clock["now"]
            cycles = ROW * len(lhs) * width / 4
            pinned = {}
            for j in range(n):
                tick(cycles, weight, calm)
                if clock["pending"] and clock["now"] >= clock["pinned"] + cfg["gap"]:
                    k = j % len(lhs)
                    pinned[k, j] = words[pl.ds(lhs[k][0] + j + zero, 1)]
                    clock["pinned"], clock["pending"] = clock["now"], False
            tiles = []
            for k, (cell, _) in enumerate(lhs):
                parts, j0 = [], 0
                for j in sorted(j for t, j in pinned if t == k):
                    parts += [words[cell + j0:cell + j]] if j > j0 else []
                    parts.append(pinned[k, j])
                    j0 = j + 1
                parts += [words[cell + j0:cell + n]] if n > j0 else []
                tiles.append(as_bf16(parts[0] if len(parts) == 1 else jnp.concatenate(parts, axis=0)))
            a = tiles[0] if len(tiles) == 1 else jnp.concatenate(tiles, axis=1)
            m = jax.lax.dot_general(a, rhs(), (((1,), (int(turn),)), ((), ())), preferred_element_type=f32)
            recent.extend((start + j * cycles, m, j * ROW) for j in range(n))
            return m

        def up_cell(c, i):
            return _BASE["weights"] + _WEIGHTS * c + 8 * i

        def down_cell(c, i):
            return up_cell(c, 55) + 9 * i

        def prep_square(src, which):
            tail = src[4 * LANE:D, :]
            tiles = [src[k * LANE:(k + 1) * LANE, :] for k in range(4)] + [jnp.concatenate([tail, tail], axis=0)]
            for k, t in enumerate(tiles):
                w = pltpu.bitcast(t.T, u32)
                square[which][D // 2 * k:D // 2 * (k + 1)] = w
                for i in range(4) if which == 1 and k == 0 else ():
                    words[_BASE["head"] + i] = w[QD // 2 * i:QD // 2 * i + 8]

        def prep_up(c):
            for r in range(0, LANE, ROW):
                for group in range(9):
                    for i, x in _right576(group, r, lambda j, k: w3_v[k:k + ROW, tile(4 * c + j)].astype(f32)):
                        put(up_cell(c, i) + r // ROW, x)
                    yield 36

        def prep_down(c):
            for r in range(0, QD, ROW):
                for b in _ORDER:
                    for i, x in _left49(b, lambda i, j: w4_v[
                            i * QD + r:i * QD + r + ROW, tile(4 * c + (j ^ 1))].astype(f32)):
                        put(down_cell(c, i) + r // ROW, x)
                    yield 40

        def columns(which):
            for j in which:
                row = sk_v[...].astype(f32)[j:j + 1] if j < 4 else (sd_v, gw_v)[j - 4][...].astype(f32).reshape(1, D)
                col_v[j] = jnp.broadcast_to(row, (LANE, D)).T

        def x_rows(u, j, r, n=ROW):
            return x_v[u][r:r + n, tile(j)].astype(f32)

        def prep_x(u):
            stats = []
            for slot, cost in enumerate((270, 230)):
                total = None
                for r in range(0, D, ROW):
                    term = [jnp.square(x_rows(u, j, r) - stats[0][j]) if stats else x_rows(u, j, r) for j in range(4)]
                    if not stats:
                        if r % QD == 0:
                            seal(col_v, cfg["lane_back"] - 100)
                        term += [t * col_v[5, r:r + ROW] for t in term]
                    total = term if total is None else [a + t for a, t in zip(total, term)]
                    if (r + ROW) % QD == 0:
                        for k in range(0, len(total), 4):
                            put(_BASE["sums"] + slot + k, (total[k] + total[k + 1]) + (total[k + 2] + total[k + 3]))
                        yield cost
                sums = [jnp.sum(a, axis=0, keepdims=True) for a in total]
                stats.append([a * (1.0 / D) for a in sums[:4]])
                for j, logit in enumerate(sums[4:]):
                    g = jax.nn.sigmoid(logit)
                    val["gate", 4 * u + j] = g
                    val["rest", 4 * u + j] = 1.0 - g
                    val["out", 4 * u + j] = (1.0 - g) * GELU_OUT
            scale = [jax.lax.rsqrt(v + LN_EPS) * GELU_IN for v in stats[1]]
            shift = [m * s for m, s in zip(stats[0], scale)]
            for r in range(0, D, ROW):
                for j in range(4):
                    put(_BASE["x"] + DC * (4 * (u % 2) + j) + r // ROW, x_rows(u, j, r) * scale[j] - shift[j])
                yield 28

        def square_product(which, source, cell):
            lhs, out = square[which], [[None] * 4 for _ in range(4)]
            for j in range(4):
                for i in range(4):
                    a = pltpu.bitcast(jnp.concatenate(
                        [lhs[(D * k + QD * i) // 2:(D * k + QD * (i + 1)) // 2] for k in range(5)], axis=1), bf16)
                    start, parts = clock["now"], []
                    for k in range(0, DC, 6):
                        tick(5 * QD / 4 / 6, cfg["room_square"])
                        first = cell + DC * j + k
                        if clock["pending"] and source is words:
                            parts += [words[pl.ds(first + zero, 1)], words[first + 1:first + 6]]
                            clock["pending"] = False
                        else:
                            parts.append(source[first:first + 6])
                    if clock["pending"] and which == 1:
                        head = pltpu.bitcast(words[pl.ds(_BASE["head"] + i + zero, 1)][0], bf16)
                        a = jnp.concatenate([jnp.concatenate([head, a[:ROW, LANE:]], axis=1), a[ROW:]], axis=0)
                        clock["pending"] = False
                    m = jnp.dot(a[:, :D], as_bf16(jnp.concatenate(parts, axis=0)), preferred_element_type=f32)
                    recent.extend((start + r * 5 / 4, m, r) for r in range(0, QD, ROW))
                    out[i][j] = m
            return out

        def mix_in(u):
            seal(arena)
            h = square_product(0, words, _BASE["x"] + 4 * DC * (u % 2))
            lane = _lane_id(QD)

            def keep(u, j, i, x):
                shifted[u][DC * j + 9 * i:DC * j + 9 * (i + 1)] = x.astype(bf16).reshape(9, ROW, LANE)

            for i, n in enumerate(SHIFTS):
                rolled = [pltpu.roll(_gelu2(z), n % LANE, 1) for z in h[i]]
                if n > 0:
                    for j in range(4):
                        before = rolled[j - 1] if j else val.get(("edge", i), 0.0)
                        keep(u, j, i, jnp.where(lane >= n, rolled[j], before))
                else:
                    if u > 0:
                        keep(u - 1, 3, i, jnp.where(lane < LANE + n, val["edge", i], rolled[0]))
                    for j in range(3 if u < NUNIT - 1 else 4):
                        keep(u, j, i, jnp.where(lane < LANE + n, rolled[j], rolled[j + 1] if j < 3 else 0.0))
                val["edge", i] = rolled[3]

        def mix_out(u):
            seal(arena)
            seal(shifted[u])
            y = square_product(1, shifted[u].bitcast(u32), 0)
            for j in range(4):
                x1, first, second = [], None, None
                for r in range(0, D, ROW):
                    i, k = divmod(r, QD)
                    x1.append(x_rows(u, j, r) + GELU_OUT * y[i][j][k:k + ROW])
                    pilot = x1[0][:1] if r == 0 else pilot
                    d = x1[-1] - pilot
                    first = d if first is None else first + d
                    second = d * d if second is None else second + d * d
                offset = jnp.sum(first, axis=0, keepdims=True) * (1.0 / D)
                var = jnp.maximum(jnp.sum(second, axis=0, keepdims=True) * (1.0 / D) - offset * offset, 0.0)
                scale = jax.lax.rsqrt(var + LN_EPS) * GELU_IN
                shift = (pilot + offset) * scale
                normal = [z * scale - shift for z in x1]
                for r, z in enumerate(x1):
                    val["skip", 4 * u + j, r] = val["rest", 4 * u + j] * z
                for k in range(5):
                    rows = normal[8 * k:8 * k + 8] if k < 4 else normal[32:] * 2
                    normed[u][5 * j + k] = jnp.concatenate(rows, axis=0).T

        def token_cell(u, i):
            return _BASE["tokens"] + 8 * (55 * u + i)

        def prep_tokens(u):
            for r in range(0, LANE, ROW):
                for group in range(9):
                    if group % 3 == 0:
                        seal(normed[u])
                    for i, x in _left576(group, lambda i, k: normed[u][5 * TILE_OF[i] + k, r:r + ROW]):
                        put(token_cell(u, i) + r // ROW, x)
                    yield 30

        def up(n, s, u, c, r):
            h = _product576(lambda a, b, k: mm([(token_cell(u, a) + r // ROW, PIECE // ROW)],
                                               lambda: as_bf16(words[up_cell(c, b):up_cell(c, b) + 8]),
                                               cfg["room_up"][k], calm=False))
            g = [[_gelu2(h[j][i ^ 1]) for j in range(4)] for i in range(4)]
            for k in range(0, PIECE, ROW):
                for p, x in _right49([[z[k:k + ROW] for z in row] for row in g]):
                    hidden[n % 2][8 * (49 * (c - FIRST[s]) + p) + (r + k) // ROW] = x.astype(bf16)
            clock["cool"] = cfg["cool"] * PIECE / 64

        def down(n, s, u, p):
            chunks = range(FIRST[s], FIRST[s + 1])
            source = hidden[n % 2].bitcast(u32)
            if p == 0:
                seal(hidden[n % 2])
                if s > 0:
                    seal(acc[u])
            m = mm([(down_cell(c, p), 9) for c in chunks],
                   lambda: jnp.concatenate([as_bf16(source[8 * (49 * k + p):8 * (49 * k + p + 1)])
                                            for k in range(len(chunks))], axis=1), cfg["room_down"], turn=True)
            if s > 0:
                m = m + acc[u][p]
            if FIRST[s + 1] == NCH:
                val["acc", u, p] = m
            else:
                acc[u][p] = m

        def finish(u, c):
            for r in range(0, QD, ROW):
                def y(b):
                    if ("outer", u, r, b) not in val:
                        val["outer", u, r, b] = _result([val["acc", u, 7 * a + b][r:r + ROW] for a in range(7)])
                    return val["outer", u, r, b]

                for i in range(2):
                    for j in range(2):
                        if c == 0:
                            rows = y(0)[i][j] + y(6)[i][j] + y(3)[i][j] - y(4)[i][j], y(3)[i][j] + y(1)[i][j]
                        else:
                            rows = y(4)[i][j] + y(2)[i][j], y(0)[i][j] - y(1)[i][j] + y(2)[i][j] + y(5)[i][j]
                        for k, z in enumerate(rows):
                            t, row = 4 * u + TILE_OF[2 * j + c], (2 * i + k) * QD + r
                            base = jnp.concatenate([val["base", t, row], val["base", t, row + 8]], axis=0)
                            out_v[row:row + ROW, tile(t)] = (base + val["out", t] * z).astype(bf16)
            if 2 * u + c + 1 in cfg["outs"]:
                copies["out", 2 * u + c + 1].start()

        def conv_cell(n, kind, rho):
            return _BASE["conv"] + 64 * (n % _RING) + 16 * kind + 4 * rho

        def conv_inputs(n):
            rows = slice(n * ROW, (n + 1) * ROW)
            lane = _lane_id(ROW // 2)
            seal(col_v, cfg["lane_back"])
            col = [col_v[j, rows] for j in range(4)]
            prev = [jnp.zeros((ROW // 2, LANE), u32)] * 3
            for i in range(NUNIT):
                seal(ssm_v, cfg["lane_back"])
                taps = _split_phases([pltpu.bitcast(ssm_v[rows, tile(4 * i + j)], u32) for j in range(4)])
                for rho in range(4):
                    words[conv_cell(n, 0, rho) + i] = taps[rho]
                yield 16
                seal(k_v, cfg["lane_back"])
                kv = []
                for t in range(4 * i, 4 * i + 4):
                    key = k_v[rows, tile(t)]
                    rolled = [pltpu.roll(pltpu.bitcast(key, u32), j, 1) for j in (1, 2, 3)]
                    total = key.astype(f32) * col[0]
                    for j in (1, 2, 3):
                        late = jnp.where(lane >= j, rolled[j - 1], prev[j - 1])
                        total = total + pltpu.bitcast(late, bf16).astype(f32) * col[j]
                    prev = rolled
                    kv.append(total * v_v[rows, tile(t)].astype(f32))
                for rho, x in enumerate(_split_phases(kv)):
                    put(conv_cell(n, 1, rho) + i, x)
                yield 140

        def conv_forward(n, kind):
            seal(arena)
            last = None
            for i in range(0, NUNIT, 2):
                u = {rho: mm([(conv_cell(n, kind, rho) + i, 2)], lambda: pltpu.bitcast(wf_v[rho], bf16),
                             cfg["room_conv"], 2) for rho in (0, 2, 1, 3)}
                for k in range(2):
                    rows = slice(k * ROW, (k + 1) * ROW)
                    z = [(u[rho][rows, :LANE], u[rho][rows, LANE:]) for rho in range(4)]
                    if kind == 0:
                        if last is None:
                            z[0] = (z[0][0] + col_v[4, n * ROW:(n + 1) * ROW], z[0][1])
                        z, last = z if last is None else [(a[0] - b[1], a[1] + b[0]) for a, b in zip(z, last)], z
                    val["spectrum", n, kind, i + k] = _dft4(z, -1)

        pairs = ((0, 3), (1, 2))

        def conv_multiply(n):
            for r in range(0, ROW, 8):
                def product(i, s):
                    re = im = None
                    for j in range(i + 1):
                        xr, xi = [z[r:r + 8] for z in val["spectrum", n, 1, j][s]]
                        kr, ki = [z[r:r + 8] for z in val["spectrum", n, 0, i - j][s]]
                        re = (xr * kr if re is None else re + xr * kr) - xi * ki
                        im = (xr * ki if im is None else im + xr * ki) + xi * kr
                    return re, im

                for h, pair in enumerate(pairs):
                    a, b = [_dft4([product(i, s) for s in range(4)], 1) for i in pair]
                    for rho in range(4):
                        for part in range(2):
                            put(conv_cell(n, 2 + part, rho) + r // 4 + h,
                                jnp.concatenate([a[rho][part], b[rho][part]], axis=0))
                    yield 185

        def conv_inverse(n):
            seal(arena)
            for k in range(2):
                ys = [mm([(conv_cell(n, 2 + part, rho) + 2 * k, 2) for part in range(2)],
                         lambda: pltpu.bitcast(wi_v[rho], bf16), cfg["room_conv"]) for rho in range(4)]
                row = n * ROW + 8 * k
                for q, i in enumerate(pairs[0] + pairs[1]):
                    y = _merge_phases([m[8 * q:8 * q + 8] for m in ys])
                    for j in range(4):
                        t = 4 * i + j
                        val["base", t, row] = ((val["gate", t] * y[j]) * x_rows(i, j, row, 8)
                                               + val["skip", t, n][8 * k:8 * k + 8])

        def job(kind, i):
            make = dict(x=prep_x, tokens=prep_tokens, up=prep_up, down=prep_down,
                        conv_in=conv_inputs, conv_mul=conv_multiply)[kind]
            return (kind, i), lambda: make(i)

        room = cfg["room_square"] * 20 * QD

        def first_stage(u, *frees):
            return lambda: mix_in(u), [("x", u)], frees, room

        def second_stage(u):
            return lambda: mix_out(u), (), [job("tokens", u)], room

        stream = [
            (lambda: wait("gw"), (), (), 0),
            (lambda: columns((5,)), (), (), 0),
            (lambda: wait(("x", 0)), (), [job("x", 0)], 0),
            (lambda: wait("w1"), [("x", 0)], (), 0),
            (lambda: prep_square(w1_v, 0), (), (), 0),
            (lambda: wait(("x", 1)), (), [job("x", 1)], 0),
            first_stage(0),
            (lambda: wait(("x", 2), ("x", 3)), (), [job("x", 2)], 0),
            first_stage(1, job("x", 3)),
            first_stage(2),
            (lambda: (wait("w2", "w3a"), prep_square(w2_v, 1)), (), [job("up", c) for c in range(FIRST[1])], 0),
            first_stage(3),
            second_stage(0),
            (lambda: wait("w4a"), (), [job("down", c) for c in range(FIRST[1])], 0),
            second_stage(1),
            second_stage(2),
            second_stage(3),
        ]

        slots = [(s, u) for s in range(len(FIRST) - 1) for u in range(NUNIT)]
        plan, begin = [], []
        for n, (s, u) in enumerate(slots):
            begin.append(len(plan))
            for c in range(FIRST[s], FIRST[s + 1]):
                for r in range(0, LANE, PIECE):
                    plan.append((len(plan) + 0.25, (
                        lambda n=n, s=s, u=u, c=c, r=r: up(n, s, u, c, r), [("up", c), ("tokens", u)], (),
                        (12 * cfg["room_up"][0] + 7 * sum(cfg["room_up"])) * PIECE / 4 - cfg["cool"] * PIECE / 64)))
        begin += [len(plan), len(plan) + 1]
        for n, (s, u) in enumerate(slots):
            count = begin[n + 2] - begin[n + 1]
            for k, p in enumerate(7 * a + b for b in _ORDER for a in range(7)):
                pos = begin[n + 1] + (k * count) // 49 + 0.5 + 0.3 * ((k * count) % 49) / 49
                plan.append((pos, (
                    lambda n=n, s=s, u=u, p=p: down(n, s, u, p),
                    [("down", c) for c in range(FIRST[s], FIRST[s + 1])] if k == 0 else (), (),
                    cfg["room_down"] * (FIRST[s + 1] - FIRST[s]) * QD / 4)))
                if FIRST[s + 1] == NCH and k in (34, 48):
                    plan.append((pos, (lambda u=u, c=int(k == 48): finish(u, c), (), (), 0)))
        plan.append((cfg["late"] + 0.1, (
            lambda: (wait("w3b", "w4b", "sk", "sd", "wf", "wi", "ssm", "k", "v"), columns(range(5))), (),
            [job(kind, c) for c in range(FIRST[1], NCH) for kind in ("up", "down")]
            + [job("conv_in", n) for n in range(2)], 0)))
        for n in range(NCONV):
            pos = round(cfg["conv"][0] + (cfg["conv"][1] - cfg["conv"][0]) * n / NCONV)
            room = cfg["room_conv"] * 8 * ROW
            frees = [job("conv_mul", n)] + [job("conv_in", m) for m in (n + 2,) if m < NCONV]
            plan += [(pos + 0.9, (lambda n=n: conv_forward(n, 0), [("conv_in", n)], (), room)),
                     (pos + 0.91, (lambda n=n: conv_forward(n, 1), (), frees, room)),
                     (pos + cfg["lag"], (lambda n=n: conv_inverse(n), [("conv_mul", n)], (), room))]
        plan.sort(key=lambda e: e[0])
        stream += [e[1] for e in plan]

        due, room_before = {}, [0.0]
        for k, (_, needs, _, room) in enumerate(stream):
            room_before.append(room_before[-1] + room)
            for name in needs:
                due.setdefault(name, k)
        for name in due:
            if name[0] in ("up", "down"):
                due[name] = min(due[name], due["conv_in", 0])
        for k, (task, needs, frees, _) in enumerate(stream):
            clock["room"] = room_before[k]
            finish_jobs(needs)
            task()
            for name, make in frees:
                jobs.append(dict(name=name, steps=make(), due=(due[name], len(jobs)), left=WORK[name[0]]))
        wait(*[("out", last) for last in cfg["outs"]])

    return kernel


def make_fn(cfg):
    def fn(A_q, A_k, A_v, A_shift_k, A_ssm_k, A_ssm_D, B_x, B_w1, B_w2, B_w3, B_w4, gate_w):
        del B_x

        def feature_major(a):
            return jnp.swapaxes(a, 1, 2).reshape(D, S)

        args = (feature_major(A_q), feature_major(A_k), feature_major(A_v), A_shift_k.T, A_ssm_k, A_ssm_D,
                B_w1, B_w2, B_w3, B_w4.T, gate_w, jnp.asarray(_WF), jnp.asarray(_WI))
        plain = pltpu.VMEM((D, S), bf16)
        marked = pltpu.VMEM((D + 2 * ROW, S), bf16)
        out = pl.pallas_call(
            _make_kernel(cfg),
            out_shape=jax.ShapeDtypeStruct((D, S), bf16),
            in_specs=[pl.BlockSpec(memory_space=pltpu.SMEM)] + [pl.BlockSpec(memory_space=pl.ANY)] * len(args),
            out_specs=pl.BlockSpec(memory_space=pl.ANY),
            scratch_shapes=[
                marked, plain, pltpu.VMEM((4, D), bf16), marked, pltpu.VMEM((D,), bf16),
                pltpu.VMEM((D, D), bf16), pltpu.VMEM((D, D), bf16),
                pltpu.VMEM((D, F), bf16), pltpu.VMEM((D, F), bf16), pltpu.VMEM((D,), bf16),
                pltpu.VMEM(_WF.shape, u32), pltpu.VMEM(_WI.shape, u32), plain,
                pltpu.VMEM((6 + 1, D, LANE), f32),
                pltpu.VMEM((_NCELL, ROW, LANE), bf16),
                pltpu.SemaphoreType.DMA((14 + NUNIT + len(cfg["outs"]),)),
                *[pltpu.VMEM((D, UNIT), bf16)] * NUNIT,
                *[pltpu.VMEM((4 * DC + 2, ROW, LANE), bf16)] * NUNIT,
                *[pltpu.VMEM((20 + 1, LANE, LANE), f32)] * NUNIT,
                *[pltpu.VMEM((49 + 1, QD, LANE), f32)] * NUNIT,
                *[pltpu.VMEM((5 * D // 2, LANE), u32)] * 2,
                *[pltpu.VMEM((4 * 49 * 8 + 2, ROW, LANE), bf16)] * 2,
            ],
            compiler_params=pltpu.CompilerParams(vmem_limit_bytes=127 * 1024 * 1024),
            name="mlp_gated_mix",
        )(jnp.asarray(np.zeros((1,), np.int32)), *args)
        return jnp.swapaxes(out.reshape(1, D, S), 1, 2)
    return fn


@jax.jit
def pallas_gated_mix__ssm_conv_h3__mixer_s_mlp__prompt_kernel(
    A_q, A_k, A_v, A_shift_k, A_ssm_k, A_ssm_D, B_x, B_w1, B_w2, B_w3, B_w4, gate_w,
):
    return make_fn(CFG)(A_q, A_k, A_v, A_shift_k, A_ssm_k, A_ssm_D, B_x, B_w1, B_w2, B_w3, B_w4, gate_w)
```
